```python
import jax
import jax.numpy as jnp

def _softmax(x, axis=-1):
    return jax.nn.softmax(x, axis=axis)

def _gelu(x):
    return jax.nn.gelu(x, approximate=True)

def _silu(x):
    return jax.nn.silu(x)

def _sigmoid(x):
    return jax.nn.sigmoid(x)

def _layernorm(x, axis=-1, eps=1e-05):
    m = jnp.mean(x, axis=axis, keepdims=True)
    v = jnp.var(x, axis=axis, keepdims=True)
    return (x - m) / jnp.sqrt(v + eps)

def _scatter_add(tgt, idx, src, axis=0):
    return tgt.at[idx].add(src)

def _segment_sum(src, seg, n):
    return jax.ops.segment_sum(src, seg, n)

class _Rng:

    def __init__(self, key):
        self._k = key

    def _next(self):
        self._k, sub = jax.random.split(self._k)
        return sub

    def normal(self, shape):
        return jax.random.normal(self._next(), shape, dtype=jnp.bfloat16)

    def randint(self, lo, hi, shape):
        return jax.random.randint(self._next(), shape, lo, hi, dtype=jnp.int32)

    def uniform(self, shape, lo=0.0, hi=1.0):
        return jax.random.uniform(self._next(), shape, jnp.bfloat16, lo, hi)

    def permutation(self, n):
        return jax.random.permutation(self._next(), n)
kernel_name = 'interleave_layers__memory_aug_recurrent_mem_tr__glu_gated_geglu__prompt'

def setup_inputs():
    _rng = _Rng(jax.random.key(int.from_bytes(__import__("os").urandom(4), "little")))
    _w = lambda a: (lambda t: t.astype(jnp.bfloat16) if jnp.issubdtype(t.dtype, jnp.floating) else t)(jnp.asarray(a))

    def _A_setup():
        B, S, Dm = (1, 2048, 1024)
        H, Dh = (32, 128)
        M, seg = (8, 32)
        seg = min(seg, S)
        S = S // seg * seg
        return {'x': _w((lambda *s: _rng.normal(s) * 0.05)(B, S, Dm)), 'mem0': _w((lambda *s: _rng.normal(s) * 0.05)(B, M, Dm)), 'Wq': _w((lambda *s: _rng.normal(s) * 0.05)(Dm, H, Dh) * Dm ** (-0.5)), 'Wk': _w((lambda *s: _rng.normal(s) * 0.05)(Dm, H, Dh) * Dm ** (-0.5)), 'Wv': _w((lambda *s: _rng.normal(s) * 0.05)(Dm, H, Dh) * Dm ** (-0.5)), 'Wo': _w((lambda *s: _rng.normal(s) * 0.05)(H, Dh, Dm) * (H * Dh) ** (-0.5)), 'seg_len': seg}
    _A_in = _A_setup()

    def _B_setup():
        B, S, Dm, Df = (1, 2048, 1024, 3584)
        return {'x': _w((lambda *s: _rng.normal(s) * 0.05)(B, S, Dm)), 'w_gate': _w((lambda *s: _rng.normal(s) * 0.05)(Dm, Df) * Dm ** (-0.5)), 'w_up': _w((lambda *s: _rng.normal(s) * 0.05)(Dm, Df) * Dm ** (-0.5)), 'w_down': _w((lambda *s: _rng.normal(s) * 0.05)(Df, Dm) * Df ** (-0.5))}
    _B_in = _B_setup()
    return {'A_x': _A_in['x'], 'A_mem0': _A_in['mem0'], 'A_Wq': _A_in['Wq'], 'A_Wk': _A_in['Wk'], 'A_Wv': _A_in['Wv'], 'A_Wo': _A_in['Wo'], 'A_seg_len': _A_in['seg_len'], 'B_x': _B_in['x'], 'B_w_gate': _B_in['w_gate'], 'B_w_up': _B_in['w_up'], 'B_w_down': _B_in['w_down']}

def reference(A_x, A_mem0, A_Wq, A_Wk, A_Wv, A_Wo, A_seg_len, B_x, B_w_gate, B_w_up, B_w_down):

    def _A_ref(x, mem0, Wq, Wk, Wv, Wo, seg_len):
        B, S, Dm = x.shape
        H, Dh = (Wq.shape[1], Wq.shape[2])
        M = mem0.shape[1]
        scale = Dh ** (-0.5)
        n_seg = S // seg_len
        L = M + seg_len
        idx = jnp.arange(L)
        mask = (idx[:, None] < M) | (idx[:, None] >= idx[None, :])
        mem = mem0
        outs = []
        for s in range(n_seg):
            xs = x[:, s * seg_len:(s + 1) * seg_len, :].copy()
            h = jnp.concatenate([mem, xs], axis=1)
            q = jnp.einsum('btd,dhe->bhte', h, Wq)
            k = jnp.einsum('btd,dhe->bhte', h, Wk)
            v = jnp.einsum('btd,dhe->bhte', h, Wv)
            scores = jnp.einsum('bhqe,bhke->bhqk', q, k) * scale
            scores = jnp.where(mask[None, None], scores, -1000000000.0)
            p = _softmax(scores, axis=-1)
            o = jnp.einsum('bhqk,bhke->bhqe', p, v)
            o = jnp.einsum('bhte,hed->btd', o, Wo)
            mem = o[:, :M, :].copy()
            outs.append(o[:, M:, :])
        return jnp.concatenate(outs, axis=1)

    def _B_ref(x, w_gate, w_up, w_down):
        g = jnp.einsum('bsd,df->bsf', x, w_gate)
        u = jnp.einsum('bsd,df->bsf', x, w_up)
        h = _gelu(g) * u
        return jnp.einsum('bsf,fd->bsd', h, w_down)
    x = A_x
    x = x + _A_ref(_layernorm(x, axis=-1), A_mem0, A_Wq, A_Wk, A_Wv, A_Wo, A_seg_len)
    x = x + _B_ref(_layernorm(x, axis=-1), B_w_gate, B_w_up, B_w_down)
    x = x + _A_ref(_layernorm(x, axis=-1), A_mem0, A_Wq, A_Wk, A_Wv, A_Wo, A_seg_len)
    x = x + _B_ref(_layernorm(x, axis=-1), B_w_gate, B_w_up, B_w_down)
    return x
```

```python
import functools

import jax
import jax.numpy as jnp
import numpy as np
import jax.experimental.pallas as pl
import jax.experimental.pallas.tpu as pltpu

F32 = jnp.float32
BF16 = jnp.bfloat16
U32 = jnp.uint32
LN_EPS = 1e-5
HG = 4
FC = 512
N_PRE = 24


def _layernorm(x):
    m = jnp.mean(x, axis=-1, keepdims=True)
    xc = x - m
    v = jnp.mean(xc * xc, axis=-1, keepdims=True)
    return xc * jax.lax.rsqrt(v + LN_EPS)


def _gelu(x):
    c = float(np.sqrt(2.0 / np.pi))
    return x * (0.5 * (1.0 + jnp.tanh(c * (x + 0.044715 * (x * x * x)))))


def _dot(a, b):
    return jnp.dot(a, b, preferred_element_type=F32)


def _dot_nt(a, b):
    return jax.lax.dot_general(a, b, (((1,), (1,)), ((), ())), preferred_element_type=F32)


def _pack(x):
    return pltpu.bitcast(x.astype(BF16), U32)


def _bf16(words):
    return pltpu.bitcast(words, BF16)


def _loop(lo, hi, fn):
    def body(i, carry):
        fn(i)
        return carry
    jax.lax.fori_loop(lo, hi, body, 0)


def _kernel(x_hbm, mem_v, wq_hbm, wk_hbm, wv_hbm, wo_hbm, wg_hbm, wu_hbm, wd_hbm,
            out_hbm,
            x_v, stage, wq, wk, wv, wo, wg, wu, wd,
            xpre, q_acc, q_pre, k_pre, v_pre, h_buf, o_buf, y_buf, z_buf, a_buf,
            keep_full, pen_full, keep_one, pen_one, keep_two, pen_two,
            out_v, x_sem, w3_sem, w_sem, out_sem,
            *, n_seg, seg, n_mem, n_heads, dh, n_pre):
    d_model = x_v.shape[1]
    d_ff = wg.shape[1]
    mt = 2 * n_mem
    half = seg // 2
    scale = float(dh) ** -0.5
    n_groups = n_heads // HG
    gw = HG * dh
    n_chunks = d_ff // FC
    dc = d_model // n_groups
    crows = dc * n_heads
    pairs = n_heads // 2
    pre0 = mt + 2 * seg
    w3 = (wq, wk, wv)
    pre = (q_pre, k_pre, v_pre)

    def get(ref, lo, hi):
        return _bf16(ref[lo // 2:hi // 2, :])

    def put(ref, lo, x):
        ref[lo // 2:(lo + x.shape[0]) // 2, :] = _pack(x)

    x_head = (2 + n_pre + 1) * seg
    x_copies = [
        pltpu.make_async_copy(x_hbm.at[lo:hi, :], x_v.at[lo:hi, :], x_sem.at[i])
        for i, (lo, hi) in enumerate(((0, x_head), (x_head, n_seg * seg)))]
    w_copies = [pltpu.make_async_copy(s.bitcast(U32), d, w_sem.at[i]) for i, (s, d) in
                enumerate(((wo_hbm, wo), (wg_hbm, wg), (wu_hbm, wu), (wd_hbm, wd)))]

    def w3_start(lo, hi):
        for i in range(lo, hi):
            m, c = divmod(i, n_groups)
            src = (wq_hbm, wk_hbm, wv_hbm)[m]
            pltpu.make_async_copy(
                src.at[c * crows:(c + 1) * crows, :], stage.at[i], w3_sem.at[i]).start()

    def w3_wait(i):
        pltpu.make_async_copy(wq_hbm.at[0:crows, :], stage.at[i], w3_sem.at[i]).wait()

    x_copies[0].start()
    w3_start(0, 2)

    stage_words = stage.bitcast(U32)

    def relayout(m, c, hp_lo=0, hp_hi=pairs):
        i = m * n_groups + c
        rows = pl.ds(pl.multiple_of(c * (dc // 2), dc // 2), dc // 2)
        for hp in range(hp_lo, hp_hi):
            a = stage_words[i, pl.ds(hp, dc // 2, stride=2 * pairs), :]
            b = stage_words[i, pl.ds(pairs + hp, dc // 2, stride=2 * pairs), :]
            g, j = divmod(2 * hp, HG)
            w3[m][g, rows, j * dh:(j + 1) * dh] = (a & U32(0xFFFF)) | (b << 16)
            w3[m][g, rows, (j + 1) * dh:(j + 2) * dh] = (a >> 16) | (b & U32(0xFFFF0000))

    def make_mask(rows, x_layers):
        qi = jax.lax.broadcasted_iota(jnp.int32, (rows, rows), 0)
        ki = jax.lax.broadcasted_iota(jnp.int32, (rows, rows), 1)

        def layer(i):
            lm = jnp.where(i < n_mem, 0, 1)
            return jnp.where(i < mt, lm, jnp.where(i < mt + seg, x_layers[0], x_layers[-1]))

        def pos(i):
            pm = jnp.where(i < n_mem, i, i - n_mem)
            px = jnp.where(i < mt + seg, i - mt, i - mt - seg) + n_mem
            return jnp.where(i < mt, pm, px)

        same = layer(qi) == layer(ki)
        causal = (pos(qi) < n_mem) | (pos(qi) >= pos(ki))
        keep = jnp.where(same & causal, 1.0, 0.0).astype(F32)
        pen = jnp.where(same, -1e9, -jnp.inf).astype(F32)
        return keep, pen

    keep_full[...], pen_full[...] = make_mask(mt + 2 * seg, (0, 1))
    keep_one[...], pen_one[...] = make_mask(mt + seg, (0,))
    keep_two[...], pen_two[...] = make_mask(mt + seg, (1,))

    def seg_rows(t):
        return pl.ds(pl.multiple_of(t * seg, seg), seg)

    def x_seg(t):
        return x_v[seg_rows(t), :].astype(F32)

    def out_copy(t, n):
        rows = pl.ds(pl.multiple_of(t * seg, seg), n * seg)
        return pltpu.make_async_copy(out_v.at[rows, :], out_hbm.at[rows, :], out_sem)

    def softmaxes(q, k, keep, pen):
        ps = []
        for j in range(HG):
            cs = slice(j * dh, (j + 1) * dh)
            s = _dot_nt(q[:, cs], k[:, cs]) * scale
            s = jnp.where(keep[...] > 0.5, s, pen[...])
            e = jnp.exp(s - jnp.max(s, axis=-1, keepdims=True))
            ps.append((e / jnp.sum(e, axis=-1, keepdims=True)).astype(BF16))
        return ps

    def weigh_values(g, ps, v):
        for j, p in enumerate(ps):
            c0 = (g * HG + j) * dh
            o = _dot(p, v[:, j * dh:(j + 1) * dh])
            o_buf[0:p.shape[0] // 2, c0:c0 + dh] = _pack(o)

    def attention(qkv, keep, pen, fillers):
        fillers = list(fillers)
        prev = None
        for g in range(n_groups + 1):
            cur = qkv(g) if g < n_groups else None
            if prev is not None:
                ps = softmaxes(prev[0], prev[1], keep, pen)
            if g > 0 and fillers:
                fillers.pop(0)()
            if prev is not None:
                weigh_values(g - 1, ps, prev[2])
            prev = cur
        for f in fillers:
            f()

    def ffn_up(yn, c):
        cs = slice(c * FC, (c + 1) * FC)
        gate = _dot(yn, _bf16(wg[:, cs]))
        up = _dot(yn, _bf16(wu[:, cs]))
        a_buf[0:yn.shape[0] // 2, cs] = _pack(_gelu(gate) * up)

    def ffn_down(rows, lo, hi):
        return _dot(get(a_buf, 0, rows), _bf16(wd[:, lo:hi]))

    def ffn_fillers(y, parts):
        yn = _layernorm(y).astype(BF16)
        split = d_model // 4

        def down(lo, hi):
            parts.append(y[:, lo:hi] + ffn_down(y.shape[0], lo, hi))

        up = [functools.partial(ffn_up, yn, c) for c in range(n_chunks)]
        return up[:-2] + [lambda: (up[-2](), up[-1]()),
                          lambda: down(0, split),
                          lambda: down(split, d_model)]

    def out_proj(rows, between=lambda: None):
        cut = d_model // 2
        o = get(o_buf, 0, rows)
        left = _dot(o, _bf16(wo[:, 0:cut]))
        between()
        return jnp.concatenate([left, _dot(o, _bf16(wo[:, cut:]))], axis=1)

    def put_mem_one_layer(r, first):
        ri = jax.lax.broadcasted_iota(jnp.int32, (mt, d_model), 0)
        act = (ri < n_mem) if first else (ri >= n_mem)
        put(h_buf, 0, jnp.where(act, r, get(h_buf, 0, mt).astype(F32)))

    def project(h, g):
        return [_dot(h, _bf16(w[g])).astype(BF16) for w in w3]

    def main_step(t, use_pre):
        if use_pre:
            h = jnp.concatenate(
                [get(h_buf, 0, mt), get(h_buf, mt + half, mt + 2 * seg)], axis=0)
            ps = pl.ds(pl.multiple_of((pre0 + (t - 2) * half) // 2, half // 2), half // 2)

            def qkv(g):
                return [jnp.concatenate([r[0:mt], _bf16(p[g, ps, :]), r[mt:]], axis=0)
                        for r, p in zip(project(h, g), pre)]
        else:
            qkv = functools.partial(project, get(h_buf, 0, mt + 2 * seg))
        z_old = z_buf[...]
        y = y_buf[...]
        put(h_buf, mt, _layernorm(x_seg(jnp.minimum(t + 1, n_seg - 1))))
        t_out = jnp.maximum(t - 3, 0)
        parts = []

        def finish():
            z = jnp.concatenate(parts, axis=1)
            z_buf[...] = z[0:seg]
            put(h_buf, mt + seg, _layernorm(z[0:seg]))
            out_v[seg_rows(t_out), :] = z[seg:2 * seg].astype(BF16)

        attention(qkv, keep_full, pen_full, ffn_fillers(y, parts))
        r = out_proj(mt + 2 * seg, finish)
        put(h_buf, 0, r[0:mt])
        y_buf[0:seg, :] = x_seg(t) + r[mt:mt + seg]
        y_buf[seg:2 * seg, :] = z_old + r[mt + seg:mt + 2 * seg]

        @pl.when(t >= 3)
        def _():
            out_copy(t_out, 1).start()

    scope = jax.named_scope
    with scope("p0_wait_x"):
        x_copies[0].wait()
    w3_start(2, 2 * n_groups)
    m0 = mem_v[...].astype(F32)
    m0 = jnp.concatenate([m0, m0], axis=0)
    put(h_buf, 0, m0)
    put(xpre, 0, m0)
    for s in range(2):
        put(xpre, mt + s * seg, _layernorm(x_seg(s)))
    for p in range(n_pre):
        lo = (2 + p) * seg
        put(xpre, pre0 + p * half, _layernorm(x_v[lo:lo + half, :].astype(F32)))
    put(h_buf, mt, _layernorm(x_seg(2)))
    y_buf[seg:2 * seg, :] = jnp.zeros((seg, d_model), F32)

    kq = 2 * dc
    n_pass = n_groups // 2

    def q_pass(s, side_work):
        xs = _bf16(xpre[:, s * kq:(s + 1) * kq])

        def group(i, part):
            g = 2 * i + part
            r = _dot(xs, _bf16(wq[g, s * kq // 2:(s + 1) * kq // 2, :]))
            if s > 0:
                r = q_acc[g] + r
            if s == n_pass - 1:
                q_pre[g] = _pack(r)
            else:
                q_acc[g] = r
            side_work(i, part)
        _loop(0, n_groups // 2, lambda i: (group(i, 0), group(i, 1)))

    with scope("p1_project_q"):
        for s in range(n_pass):
            for c in (2 * s, 2 * s + 1):
                w3_wait(c)
                relayout(0, c)
            if s == 1:
                w3_start(2 * n_groups, 3 * n_groups)
            if s == n_pass - 1:
                for c in range(n_groups // 2):
                    w3_wait(n_groups + c)
                q_pass(s, lambda c, j: relayout(1, c, j * pairs // 2, (j + 1) * pairs // 2))
            else:
                q_pass(s, lambda c, j: None)

    def project_group(m, g, side_work=lambda j: None):
        xs = _bf16(xpre[...])
        for j in range(HG):
            cs = slice(j * dh, (j + 1) * dh)
            side_work(j)
            pre[m][g, :, cs] = _pack(_dot(xs, _bf16(w3[m][g, :, cs])))

    def relayout_part(m, c, j):
        relayout(m, c, j * pairs // HG, (j + 1) * pairs // HG)

    with scope("p2_relayout_k"):
        w_copies[0].start()
        for c in range(n_groups // 2, n_groups):
            w3_wait(n_groups + c)
            relayout(1, c)
    with scope("p3_project_k"):
        _loop(0, n_groups // 2, lambda g: project_group(1, g))
        w_copies[1].start()
        for c in range(n_groups):
            w3_wait(2 * n_groups + c)

        def k_and_relayout(g):
            c = 2 * (g - n_groups // 2)
            project_group(1, g, lambda j: (relayout_part(2, c, j), relayout_part(2, c + 1, j)))

        _loop(n_groups // 2, n_groups, k_and_relayout)
    w_copies[2].start()
    w_copies[3].start()
    x_copies[1].start()
    with scope("p4_project_v"):
        _loop(0, n_groups, lambda g: project_group(2, g))

    def precomputed(g, lo, hi):
        return [_bf16(p[g, lo // 2:hi // 2, :]) for p in pre]

    with scope("p5_seg0"):
        w_copies[0].wait()
        attention(lambda g: precomputed(g, 0, mt + seg), keep_one, pen_one, [])
        r = out_proj(mt + seg)
        put_mem_one_layer(r[0:mt], True)
        y_buf[0:seg, :] = x_seg(0) + r[mt:]

    with scope("p6_seg1"):
        hm = get(h_buf, 0, mt)
        attention(
            lambda g: [jnp.concatenate(mp, axis=0) for mp in
                       zip(project(hm, g), precomputed(g, mt + seg, mt + 2 * seg))],
            keep_one, pen_one, [])
        r = out_proj(mt + seg)
        put_mem_one_layer(r[0:mt], True)
        z_buf[...] = x_seg(1) + r[mt:]

    with scope("p7_ffn0"):
        w_copies[1].wait()
        w_copies[2].wait()
        w_copies[3].wait()
        y = y_buf[0:seg, :]
        yn = _layernorm(y).astype(BF16)
        for c in range(n_chunks):
            ffn_up(yn, c)
        z = y + ffn_down(seg, 0, d_model)
        y_buf[0:seg, :] = z_buf[...]
        z_buf[...] = z
        put(h_buf, mt + seg, _layernorm(z))

    with scope("p8_main_pre"):
        _loop(2, 2 + n_pre, lambda t: main_step(t, True))
    x_copies[1].wait()
    with scope("p9_main"):
        _loop(2 + n_pre, n_seg, lambda t: main_step(t, False))

    def second_layer_only(with_ffn):
        h = jnp.concatenate(
            [get(h_buf, 0, mt), get(h_buf, mt + seg, mt + 2 * seg)], axis=0)
        z_old = z_buf[...]
        parts = []

        def finish():
            z = jnp.concatenate(parts, axis=1)
            z_buf[...] = z[0:seg]
            put(h_buf, mt + seg, _layernorm(z[0:seg]))
            out_v[(n_seg - 3) * seg:(n_seg - 2) * seg, :] = z[seg:2 * seg].astype(BF16)

        attention(functools.partial(project, h), keep_two, pen_two,
                  ffn_fillers(y_buf[...], parts) if with_ffn else [])
        if with_ffn:
            r = out_proj(mt + seg, finish)
            put_mem_one_layer(r[0:mt], False)
            y_buf[0:seg, :] = z_old + r[mt:]
            out_copy(n_seg - 3, 1).start()
        else:
            y_buf[seg:2 * seg, :] = z_old + out_proj(mt + seg)[mt:]

    with scope("pa_e0"):
        second_layer_only(True)
    with scope("pb_e1"):
        second_layer_only(False)
    with scope("pc_e2"):
        y = y_buf[...]
        yn = _layernorm(y).astype(BF16)
        for c in range(n_chunks):
            ffn_up(yn, c)
        z = y + ffn_down(2 * seg, 0, d_model)
        out_v[(n_seg - 2) * seg:n_seg * seg, :] = z.astype(BF16)
        out_copy(n_seg - 2, 2).start()
        pltpu.make_async_copy(out_v, out_hbm, out_sem).wait()


@functools.partial(jax.jit, static_argnames=("A_seg_len",))
def pallas_interleave_layers__memory_aug_recurrent_mem_tr__glu_gated_geglu__prompt_kernel(
    A_x, A_mem0, A_Wq, A_Wk, A_Wv, A_Wo, A_seg_len, B_x, B_w_gate, B_w_up, B_w_down,
):
    del B_x
    _, S, Dm = A_x.shape
    _, M, _ = A_mem0.shape
    _, H, Dh = A_Wq.shape
    Df = B_w_gate.shape[1]
    seg = int(A_seg_len)
    n_seg = S // seg
    mt = 2 * M
    G = H // HG
    gw = HG * Dh
    rows = mt + 2 * seg
    pre_rows = rows + N_PRE * (seg // 2)

    kern = functools.partial(
        _kernel, n_seg=n_seg, seg=seg, n_mem=M, n_heads=H, dh=Dh, n_pre=N_PRE)
    any_spec = pl.BlockSpec(memory_space=pl.ANY)
    out = pl.pallas_call(
        kern,
        in_specs=[any_spec, pl.BlockSpec(memory_space=pltpu.VMEM)] + [any_spec] * 7,
        out_specs=any_spec,
        out_shape=jax.ShapeDtypeStruct((S, Dm), A_x.dtype),
        scratch_shapes=[
            pltpu.VMEM((S, Dm), BF16),
            pltpu.VMEM((3 * G, Dm // G * H, Dh), BF16),
            pltpu.VMEM((G, Dm // 2, gw), U32),
            pltpu.VMEM((G, Dm // 2, gw), U32),
            pltpu.VMEM((G, Dm // 2, gw), U32),
            pltpu.VMEM((H * Dh // 2, Dm), U32),
            pltpu.VMEM((Dm // 2, Df), U32),
            pltpu.VMEM((Dm // 2, Df), U32),
            pltpu.VMEM((Df // 2, Dm), U32),
            pltpu.VMEM((pre_rows // 2, Dm), U32),
            pltpu.VMEM((G, pre_rows, gw), F32),
            pltpu.VMEM((G, pre_rows // 2, gw), U32),
            pltpu.VMEM((G, pre_rows // 2, gw), U32),
            pltpu.VMEM((G, pre_rows // 2, gw), U32),
            pltpu.VMEM((rows // 2, Dm), U32),
            pltpu.VMEM((rows // 2, H * Dh), U32),
            pltpu.VMEM((2 * seg, Dm), F32),
            pltpu.VMEM((seg, Dm), F32),
            pltpu.VMEM((seg, Df), U32),
            pltpu.VMEM((rows, rows), F32),
            pltpu.VMEM((rows, rows), F32),
            pltpu.VMEM((mt + seg, mt + seg), F32),
            pltpu.VMEM((mt + seg, mt + seg), F32),
            pltpu.VMEM((mt + seg, mt + seg), F32),
            pltpu.VMEM((mt + seg, mt + seg), F32),
            pltpu.VMEM((S, Dm), BF16),
            pltpu.SemaphoreType.DMA((2,)),
            pltpu.SemaphoreType.DMA((3 * G,)),
            pltpu.SemaphoreType.DMA((4,)),
            pltpu.SemaphoreType.DMA(()),
        ],
        compiler_params=pltpu.CompilerParams(vmem_limit_bytes=124 * 1024 * 1024),
    )(
        A_x.reshape(S, Dm), A_mem0.reshape(M, Dm),
        A_Wq.reshape(Dm * H, Dh), A_Wk.reshape(Dm * H, Dh), A_Wv.reshape(Dm * H, Dh),
        A_Wo.reshape(H * Dh, Dm), B_w_gate, B_w_up, B_w_down,
    )
    return out.reshape(1, S, Dm)
```

```python
import functools

import jax
import jax.numpy as jnp
import numpy as np
import jax.experimental.pallas as pl
import jax.experimental.pallas.tpu as pltpu

F32 = jnp.float32
BF16 = jnp.bfloat16
U32 = jnp.uint32
LN_EPS = 1e-5
HG = 4
FC = 512
N_PRE = 11


def _layernorm(x):
    m = jnp.mean(x, axis=-1, keepdims=True)
    xc = x - m
    v = jnp.mean(xc * xc, axis=-1, keepdims=True)
    return xc * jax.lax.rsqrt(v + LN_EPS)


def _gelu(x):
    c = float(np.sqrt(2.0 / np.pi))
    return x * (0.5 * (1.0 + jnp.tanh(c * (x + 0.044715 * (x * x * x)))))


def _dot(a, b):
    return jnp.dot(a, b, preferred_element_type=F32)


def _dot_nt(a, b):
    return jax.lax.dot_general(a, b, (((1,), (1,)), ((), ())), preferred_element_type=F32)


def _pack(x):
    return pltpu.bitcast(x.astype(BF16), U32)


def _bf16(words):
    return pltpu.bitcast(words, BF16)


def _loop(lo, hi, fn):
    def body(i, carry):
        fn(i)
        return carry
    jax.lax.fori_loop(lo, hi, body, 0)


def _kernel(x_hbm, mem_v, wq_hbm, wk_hbm, wv_hbm, wo_hbm, wg_hbm, wu_hbm, wd_hbm,
            out_hbm,
            x_v, stage, wq, wk, wv, wo, wg, wu, wd,
            xpre, q_acc, q_pre, k_pre, v_pre, h_buf, o_buf, y_buf, z_buf, a_buf,
            keep_full, pen_full, keep_one, pen_one, keep_two, pen_two,
            out_v, x_sem, w3_sem, w_sem, out_sem,
            *, n_seg, seg, n_mem, n_heads, dh, n_pre):
    d_model = x_v.shape[1]
    d_ff = wg.shape[1]
    mt = 2 * n_mem
    scale = float(dh) ** -0.5
    n_groups = n_heads // HG
    gw = HG * dh
    n_chunks = d_ff // FC
    dc = d_model // n_groups
    crows = dc * n_heads
    pairs = n_heads // 2
    w3 = (wq, wk, wv)
    pre = (q_pre, k_pre, v_pre)

    def get(ref, lo, hi):
        return _bf16(ref[lo // 2:hi // 2, :])

    def put(ref, lo, x):
        ref[lo // 2:(lo + x.shape[0]) // 2, :] = _pack(x)

    x_head = (2 + n_pre + 1) * seg
    x_copies = [
        pltpu.make_async_copy(x_hbm.at[lo:hi, :], x_v.at[lo:hi, :], x_sem.at[i])
        for i, (lo, hi) in enumerate(((0, x_head), (x_head, n_seg * seg)))]
    w_copies = [pltpu.make_async_copy(s.bitcast(U32), d, w_sem.at[i]) for i, (s, d) in
                enumerate(((wo_hbm, wo), (wg_hbm, wg), (wu_hbm, wu), (wd_hbm, wd)))]

    def w3_start(lo, hi):
        for i in range(lo, hi):
            m, c = divmod(i, n_groups)
            src = (wq_hbm, wk_hbm, wv_hbm)[m]
            pltpu.make_async_copy(
                src.at[c * crows:(c + 1) * crows, :], stage.at[i], w3_sem.at[i]).start()

    def w3_wait(i):
        pltpu.make_async_copy(wq_hbm.at[0:crows, :], stage.at[i], w3_sem.at[i]).wait()

    x_copies[0].start()
    w3_start(0, 1)

    stage_words = stage.bitcast(U32)

    def relayout(m, c, hp_lo=0, hp_hi=pairs):
        i = m * n_groups + c
        rows = pl.ds(pl.multiple_of(c * (dc // 2), dc // 2), dc // 2)
        for hp in range(hp_lo, hp_hi):
            a = stage_words[i, pl.ds(hp, dc // 2, stride=2 * pairs), :]
            b = stage_words[i, pl.ds(pairs + hp, dc // 2, stride=2 * pairs), :]
            g, j = divmod(2 * hp, HG)
            w3[m][g, rows, j * dh:(j + 1) * dh] = (a & U32(0xFFFF)) | (b << 16)
            w3[m][g, rows, (j + 1) * dh:(j + 2) * dh] = (a >> 16) | (b & U32(0xFFFF0000))

    def make_mask(rows, x_layers):
        qi = jax.lax.broadcasted_iota(jnp.int32, (rows, rows), 0)
        ki = jax.lax.broadcasted_iota(jnp.int32, (rows, rows), 1)

        def layer(i):
            lm = jnp.where(i < n_mem, 0, 1)
            return jnp.where(i < mt, lm, jnp.where(i < mt + seg, x_layers[0], x_layers[-1]))

        def pos(i):
            pm = jnp.where(i < n_mem, i, i - n_mem)
            px = jnp.where(i < mt + seg, i - mt, i - mt - seg) + n_mem
            return jnp.where(i < mt, pm, px)

        same = layer(qi) == layer(ki)
        causal = (pos(qi) < n_mem) | (pos(qi) >= pos(ki))
        keep = jnp.where(same & causal, 1.0, 0.0).astype(F32)
        pen = jnp.where(same, -1e9, -jnp.inf).astype(F32)
        return keep, pen

    keep_full[...], pen_full[...] = make_mask(mt + 2 * seg, (0, 1))
    keep_one[...], pen_one[...] = make_mask(mt + seg, (0,))
    keep_two[...], pen_two[...] = make_mask(mt + seg, (1,))

    def seg_rows(t):
        return pl.ds(pl.multiple_of(t * seg, seg), seg)

    def x_seg(t):
        return x_v[seg_rows(t), :].astype(F32)

    def out_copy(t, n):
        rows = pl.ds(pl.multiple_of(t * seg, seg), n * seg)
        return pltpu.make_async_copy(out_v.at[rows, :], out_hbm.at[rows, :], out_sem)

    def softmaxes(q, k, keep, pen):
        ps = []
        for j in range(HG):
            cs = slice(j * dh, (j + 1) * dh)
            s = _dot_nt(q[:, cs], k[:, cs]) * scale
            s = jnp.where(keep[...] > 0.5, s, pen[...])
            e = jnp.exp(s - jnp.max(s, axis=-1, keepdims=True))
            ps.append((e / jnp.sum(e, axis=-1, keepdims=True)).astype(BF16))
        return ps

    def weigh_values(g, ps, v):
        for j, p in enumerate(ps):
            o = _dot(p, v[:, j * dh:(j + 1) * dh])
            o_buf[g, 0:p.shape[0] // 2, j * dh:(j + 1) * dh] = _pack(o)

    def attention(qkv, keep, pen, fillers):
        fillers = list(fillers)
        ready = [qkv(0), qkv(1)]
        for g in range(n_groups):
            q, k, v = ready[g]
            ps = softmaxes(q, k, keep, pen)
            if g + 2 < n_groups:
                ready.append(qkv(g + 2))
            if fillers:
                fillers.pop(0)()
            weigh_values(g, ps, v)
        for f in fillers:
            f()

    def ffn_up(yn, c):
        cs = slice(c * FC, (c + 1) * FC)
        gate = _dot(yn, _bf16(wg[:, cs]))
        up = _dot(yn, _bf16(wu[:, cs]))
        a_buf[0:yn.shape[0] // 2, cs] = _pack(_gelu(gate) * up)

    def ffn_down(rows, lo, hi):
        return _dot(get(a_buf, 0, rows), _bf16(wd[:, lo:hi]))

    def ffn_fillers(y, parts):
        yn = _layernorm(y).astype(BF16)
        split = d_model // 4

        def down(lo, hi):
            parts.append(y[:, lo:hi] + ffn_down(y.shape[0], lo, hi))

        up = [functools.partial(ffn_up, yn, c) for c in range(n_chunks)]
        return up[:-2] + [lambda: (up[-2](), up[-1]()),
                          lambda: down(0, split),
                          lambda: down(split, d_model)]

    def out_proj(rows, between=lambda: None):
        cut = d_model // 2
        o = jnp.concatenate(
            [_bf16(o_buf[g, 0:rows // 2, :]) for g in range(n_groups)], axis=1)
        left = _dot(o, _bf16(wo[:, 0:cut]))
        between()
        return jnp.concatenate([left, _dot(o, _bf16(wo[:, cut:]))], axis=1)

    def put_mem_one_layer(r, first):
        ri = jax.lax.broadcasted_iota(jnp.int32, (mt, d_model), 0)
        act = (ri < n_mem) if first else (ri >= n_mem)
        put(h_buf, 0, jnp.where(act, r, get(h_buf, 0, mt).astype(F32)))

    def project(h, g):
        return [_dot(h, _bf16(w[g])).astype(BF16) for w in w3]

    def main_step(t, use_pre):
        if use_pre:
            h = jnp.concatenate(
                [get(h_buf, 0, mt), get(h_buf, mt + seg, mt + 2 * seg)], axis=0)
            ps = pl.ds(pl.multiple_of((mt + t * seg) // 2, mt // 2), seg // 2)

            def qkv(g):
                return [jnp.concatenate([r[0:mt], _bf16(p[g, ps, :]), r[mt:]], axis=0)
                        for r, p in zip(project(h, g), pre)]
        else:
            qkv = functools.partial(project, get(h_buf, 0, mt + 2 * seg))
        z_old = z_buf[...]
        y = y_buf[...]
        if not use_pre:
            put(h_buf, mt, _layernorm(x_seg(jnp.minimum(t + 1, n_seg - 1))))
        t_out = jnp.maximum(t - 3, 0)
        parts = []

        def finish():
            z = jnp.concatenate(parts, axis=1)
            z_buf[...] = z[0:seg]
            put(h_buf, mt + seg, _layernorm(z[0:seg]))
            out_v[seg_rows(t_out), :] = z[seg:2 * seg].astype(BF16)

        attention(qkv, keep_full, pen_full, ffn_fillers(y, parts))
        r = out_proj(mt + 2 * seg, finish)
        put(h_buf, 0, r[0:mt])
        y_buf[0:seg, :] = x_seg(t) + r[mt:mt + seg]
        y_buf[seg:2 * seg, :] = z_old + r[mt + seg:mt + 2 * seg]

        @pl.when(t >= 3)
        def _():
            out_copy(t_out, 1).start()

    scope = jax.named_scope
    with scope("p0_wait_x"):
        x_copies[0].wait()
    w3_start(1, 2 * n_groups)
    m0 = mem_v[...].astype(F32)
    m0 = jnp.concatenate([m0, m0], axis=0)
    put(h_buf, 0, m0)
    put(xpre, 0, m0)
    for s in range(2 + n_pre):
        put(xpre, mt + s * seg, _layernorm(x_seg(s)))
    put(h_buf, mt, _layernorm(x_seg(2 + n_pre)))
    y_buf[seg:2 * seg, :] = jnp.zeros((seg, d_model), F32)

    def relayout_part(m, c, j, n):
        relayout(m, c, j * pairs // n, (j + 1) * pairs // n)

    kq = d_model // 2
    nq = n_groups // 2
    side = [[], [(0, nq)], [(0, nq + 1), (0, nq + 2)], [(0, nq + 3), (1, 0)],
            [(1, 1), (1, 2)], [(1, 3), (1, 4)], [(1, 5)], [(1, 6), (1, 7)]]
    assert n_groups == 8
    with scope("p1_project_q"):
        for c in range(nq):
            w3_wait(c)
            relayout(0, c)
        for step, chunks in enumerate(side):
            s, i = divmod(step, nq)
            if step == nq:
                w3_start(2 * n_groups, 3 * n_groups)
            for m, c in chunks:
                w3_wait(m * n_groups + c)
            xs = _bf16(xpre[:, s * kq:(s + 1) * kq])
            for part in range(4):
                g, cs = 2 * i + part // 2, slice(part % 2 * gw // 2, (part % 2 + 1) * gw // 2)
                for m, c in chunks:
                    relayout_part(m, c, part, 4)
                r = _dot(xs, _bf16(wq[g, s * kq // 2:(s + 1) * kq // 2, cs]))
                if s == 0:
                    q_acc[g, :, cs] = r
                else:
                    q_pre[g, :, cs] = _pack(q_acc[g, :, cs] + r)

    def project_group(m, g, side_work=lambda j: None):
        xs = _bf16(xpre[...])
        for j in range(HG):
            cs = slice(j * dh, (j + 1) * dh)
            side_work(j)
            pre[m][g, :, cs] = _pack(_dot(xs, _bf16(w3[m][g, :, cs])))

    def precomputed(p, g, lo, hi):
        return _bf16(p[g, lo // 2:hi // 2, :])

    def k_group(g):
        w3_wait(2 * n_groups + g)
        project_group(1, g, lambda j: relayout_part(2, g, j, HG))

    def v_group(g):
        ps = softmaxes(precomputed(q_pre, g, 0, mt + seg), precomputed(k_pre, g, 0, mt + seg),
                       keep_one, pen_one)
        project_group(2, g)
        weigh_values(g, ps, precomputed(v_pre, g, 0, mt + seg))

    w_copies[0].start()
    w_copies[1].start()
    with scope("p3_project_k"):
        _loop(0, n_groups, k_group)
    w_copies[2].start()
    w_copies[3].start()
    x_copies[1].start()
    with scope("p4_project_v"):
        _loop(0, n_groups, v_group)

    with scope("p5_seg0"):
        w_copies[0].wait()
        r = out_proj(mt + seg)
        put_mem_one_layer(r[0:mt], True)
        y_buf[0:seg, :] = x_seg(0) + r[mt:]

    with scope("p6_seg1"):
        w_copies[1].wait()
        w_copies[2].wait()
        hm = get(h_buf, 0, mt)
        yn = _layernorm(y_buf[0:seg, :]).astype(BF16)
        attention(
            lambda g: [jnp.concatenate([r, precomputed(p, g, mt + seg, mt + 2 * seg)], axis=0)
                       for r, p in zip(project(hm, g), pre)],
            keep_one, pen_one, [functools.partial(ffn_up, yn, c) for c in range(n_chunks)])
        r = out_proj(mt + seg)
        put_mem_one_layer(r[0:mt], True)
        z_buf[...] = x_seg(1) + r[mt:]

    with scope("p7_ffn0"):
        w_copies[3].wait()
        z = y_buf[0:seg, :] + ffn_down(seg, 0, d_model)
        y_buf[0:seg, :] = z_buf[...]
        z_buf[...] = z
        put(h_buf, mt + seg, _layernorm(z))

    with scope("p8_main_pre"):
        _loop(2, 2 + n_pre, lambda t: main_step(t, True))
    x_copies[1].wait()
    with scope("p9_main"):
        _loop(2 + n_pre, n_seg, lambda t: main_step(t, False))

    def second_layer_only(t):
        first = t == n_seg
        h = jnp.concatenate(
            [get(h_buf, 0, mt), get(h_buf, mt + seg, mt + 2 * seg)], axis=0)
        z_old = z_buf[...]
        parts = []

        def finish():
            z = jnp.concatenate(parts, axis=1)
            if first:
                z_buf[...] = z[0:seg]
                put(h_buf, mt + seg, _layernorm(z[0:seg]))
            out_v[(t - 3) * seg:(t - 2) * seg, :] = z[z.shape[0] - seg:].astype(BF16)

        attention(functools.partial(project, h), keep_two, pen_two,
                  ffn_fillers(y_buf[0 if first else seg:2 * seg, :], parts))
        r = out_proj(mt + seg, finish)
        if first:
            put_mem_one_layer(r[0:mt], False)
        y_buf[seg:2 * seg, :] = z_old + r[mt:]
        out_copy(t - 3, 1).start()

    with scope("pa_e0"):
        second_layer_only(n_seg)
    with scope("pb_e1"):
        second_layer_only(n_seg + 1)
    with scope("pc_e2"):
        y = y_buf[seg:2 * seg, :]
        yn = _layernorm(y).astype(BF16)
        for c in range(n_chunks):
            ffn_up(yn, c)
        z = y + ffn_down(seg, 0, d_model)
        out_v[(n_seg - 1) * seg:n_seg * seg, :] = z.astype(BF16)
        out_copy(n_seg - 1, 1).start()
        pltpu.make_async_copy(out_v, out_hbm, out_sem).wait()


@functools.partial(jax.jit, static_argnames=("A_seg_len",))
def pallas_interleave_layers__memory_aug_recurrent_mem_tr__glu_gated_geglu__prompt_kernel(
    A_x, A_mem0, A_Wq, A_Wk, A_Wv, A_Wo, A_seg_len, B_x, B_w_gate, B_w_up, B_w_down,
):
    del B_x
    _, S, Dm = A_x.shape
    _, M, _ = A_mem0.shape
    _, H, Dh = A_Wq.shape
    Df = B_w_gate.shape[1]
    seg = int(A_seg_len)
    n_seg = S // seg
    mt = 2 * M
    G = H // HG
    gw = HG * Dh
    rows = mt + 2 * seg
    pre_rows = mt + (2 + N_PRE) * seg

    kern = functools.partial(
        _kernel, n_seg=n_seg, seg=seg, n_mem=M, n_heads=H, dh=Dh, n_pre=N_PRE)
    any_spec = pl.BlockSpec(memory_space=pl.ANY)
    out = pl.pallas_call(
        kern,
        in_specs=[any_spec, pl.BlockSpec(memory_space=pltpu.VMEM)] + [any_spec] * 7,
        out_specs=any_spec,
        out_shape=jax.ShapeDtypeStruct((S, Dm), A_x.dtype),
        scratch_shapes=[
            pltpu.VMEM((S, Dm), BF16),
            pltpu.VMEM((3 * G, Dm // G * H, Dh), BF16),
            pltpu.VMEM((G, Dm // 2, gw), U32),
            pltpu.VMEM((G, Dm // 2, gw), U32),
            pltpu.VMEM((G, Dm // 2, gw), U32),
            pltpu.VMEM((H * Dh // 2, Dm), U32),
            pltpu.VMEM((Dm // 2, Df), U32),
            pltpu.VMEM((Dm // 2, Df), U32),
            pltpu.VMEM((Df // 2, Dm), U32),
            pltpu.VMEM((pre_rows // 2, Dm), U32),
            pltpu.VMEM((G, pre_rows, gw), F32),
            pltpu.VMEM((G, pre_rows // 2, gw), U32),
            pltpu.VMEM((G, pre_rows // 2, gw), U32),
            pltpu.VMEM((G, pre_rows // 2, gw), U32),
            pltpu.VMEM((rows // 2, Dm), U32),
            pltpu.VMEM((G, rows // 2, gw), U32),
            pltpu.VMEM((2 * seg, Dm), F32),
            pltpu.VMEM((seg, Dm), F32),
            pltpu.VMEM((seg, Df), U32),
            pltpu.VMEM((rows, rows), F32),
            pltpu.VMEM((rows, rows), F32),
            pltpu.VMEM((mt + seg, mt + seg), F32),
            pltpu.VMEM((mt + seg, mt + seg), F32),
            pltpu.VMEM((mt + seg, mt + seg), F32),
            pltpu.VMEM((mt + seg, mt + seg), F32),
            pltpu.VMEM((S, Dm), BF16),
            pltpu.SemaphoreType.DMA((2,)),
            pltpu.SemaphoreType.DMA((3 * G,)),
            pltpu.SemaphoreType.DMA((4,)),
            pltpu.SemaphoreType.DMA(()),
        ],
        compiler_params=pltpu.CompilerParams(vmem_limit_bytes=124 * 1024 * 1024),
    )(
        A_x.reshape(S, Dm), A_mem0.reshape(M, Dm),
        A_Wq.reshape(Dm * H, Dh), A_Wk.reshape(Dm * H, Dh), A_Wv.reshape(Dm * H, Dh),
        A_Wo.reshape(H * Dh, Dm), B_w_gate, B_w_up, B_w_down,
    )
    return out.reshape(1, S, Dm)
```

```python
import functools

import jax
import jax.numpy as jnp
import numpy as np
import jax.experimental.pallas as pl
import jax.experimental.pallas.tpu as pltpu

F32 = jnp.float32
BF16 = jnp.bfloat16
U32 = jnp.uint32
LN_EPS = 1e-5
HG = 4
FC = 512
N_PRE = 11


def _layernorm(x):
    m = jnp.mean(x, axis=-1, keepdims=True)
    xc = x - m
    v = jnp.mean(xc * xc, axis=-1, keepdims=True)
    return xc * jax.lax.rsqrt(v + LN_EPS)


def _gelu(x):
    c = float(np.sqrt(2.0 / np.pi))
    return x * (0.5 * (1.0 + jnp.tanh(c * (x + 0.044715 * (x * x * x)))))


def _dot(a, b):
    return jnp.dot(a, b, preferred_element_type=F32)


def _dot_nt(a, b):
    return jax.lax.dot_general(a, b, (((1,), (1,)), ((), ())), preferred_element_type=F32)


def _pack(x):
    return pltpu.bitcast(x.astype(BF16), U32)


def _bf16(words):
    return pltpu.bitcast(words, BF16)


def _loop(lo, hi, fn, unroll=1, first=None):
    assert (hi - lo) % unroll == 0

    def body(i, carry):
        steps = [lo + i * unroll + u for u in range(unroll)]
        for stage in ((first, fn) if first else (fn,)):
            for t in steps:
                stage(t)
        return carry
    jax.lax.fori_loop(0, (hi - lo) // unroll, body, 0)


def _kernel(x_hbm, mem_v, wq_hbm, wk_hbm, wv_hbm, wo_hbm, wg_hbm, wu_hbm, wd_hbm,
            out_hbm,
            x_v, stage, tmp, wq, wk, wv, wo, wg, wu, wd,
            xpre, q_acc, q_pre, k_pre, v_pre, h_buf, o_buf, y_buf, z_buf, a_buf,
            keep_full, pen_full, keep_one, pen_one, keep_two, pen_two,
            out_v, x_sem, w3_sem, w_sem, out_sem,
            *, n_seg, seg, n_mem, n_heads, dh, n_pre):
    d_model = x_v.shape[1]
    d_ff = wg.shape[1]
    mt = 2 * n_mem
    scale = float(dh) ** -0.5
    half = seg // 2
    pre0 = mt + seg + half
    n_groups = n_heads // HG
    gw = HG * dh
    n_chunks = d_ff // FC
    dc = d_model // n_groups
    crows = dc * n_heads
    pairs = n_heads // 2
    w3 = (wq, wk, wv)
    pre = (q_pre, k_pre, v_pre)

    def get(ref, lo, hi):
        return _bf16(ref[lo // 2:hi // 2, :])

    def put(ref, lo, x):
        ref[lo // 2:(lo + x.shape[0]) // 2, :] = _pack(x)

    x_head = (2 + n_pre + 1) * seg
    x_copies = [
        pltpu.make_async_copy(x_hbm.at[lo:hi, :], x_v.at[lo:hi, :], x_sem.at[i])
        for i, (lo, hi) in enumerate(((0, x_head), (x_head, n_seg * seg)))]
    w_copies = [pltpu.make_async_copy(s.bitcast(U32), d, w_sem.at[i]) for i, (s, d) in
                enumerate(((wo_hbm, wo), (wg_hbm, wg), (wu_hbm, wu), (wd_hbm, wd)))]

    def w3_start(lo, hi):
        for i in range(lo, hi):
            m, c = divmod(i, n_groups)
            src = (wq_hbm, wk_hbm, wv_hbm)[m]
            pltpu.make_async_copy(
                src.at[c * crows:(c + 1) * crows, :], stage.at[i], w3_sem.at[i]).start()

    def w3_wait(i):
        pltpu.make_async_copy(wq_hbm.at[0:crows, :], stage.at[i], w3_sem.at[i]).wait()

    x_copies[0].start()
    w3_start(0, 1)

    stage_words = stage.bitcast(U32)

    def relayout(m, c, q_lo=0, q_hi=4):
        i = m * n_groups + c
        rows = pl.ds(pl.multiple_of(c * (dc // 2), dc // 2), dc // 2)
        for lo in range(q_lo, q_hi):
            tmp[lo] = stage_words[i, pl.ds(lo, dc * pairs // 4, stride=4), :]
            for a in range(pairs // 4):
                even = tmp[lo, pl.ds(a, dc // 2, stride=pairs // 2), :]
                odd = tmp[lo, pl.ds(pairs // 4 + a, dc // 2, stride=pairs // 2), :]
                g, j = divmod(2 * (4 * a + lo), HG)
                w3[m][g, rows, j * dh:(j + 1) * dh] = (even & U32(0xFFFF)) | (odd << 16)
                w3[m][g, rows, (j + 1) * dh:(j + 2) * dh] = (
                    (even >> 16) | (odd & U32(0xFFFF0000)))

    def make_mask(rows, x_layers):
        qi = jax.lax.broadcasted_iota(jnp.int32, (rows, rows), 0)
        ki = jax.lax.broadcasted_iota(jnp.int32, (rows, rows), 1)

        def layer(i):
            lm = jnp.where(i < n_mem, 0, 1)
            return jnp.where(i < mt, lm, jnp.where(i < mt + seg, x_layers[0], x_layers[-1]))

        def pos(i):
            pm = jnp.where(i < n_mem, i, i - n_mem)
            px = jnp.where(i < mt + seg, i - mt, i - mt - seg) + n_mem
            return jnp.where(i < mt, pm, px)

        same = layer(qi) == layer(ki)
        causal = (pos(qi) < n_mem) | (pos(qi) >= pos(ki))
        keep = jnp.where(same & causal, 1.0, 0.0).astype(F32)
        pen = jnp.where(same, -1e9, -jnp.inf).astype(F32)
        return keep, pen

    keep_full[...], pen_full[...] = make_mask(mt + 2 * seg, (0, 1))
    keep_one[...], pen_one[...] = make_mask(mt + seg, (0,))
    keep_two[...], pen_two[...] = make_mask(mt + seg, (1,))

    def seg_rows(t):
        return pl.ds(pl.multiple_of(t * seg, seg), seg)

    def x_seg(t):
        return x_v[seg_rows(t), :].astype(F32)

    def out_copy(t, n):
        rows = pl.ds(pl.multiple_of(t * seg, seg), n * seg)
        return pltpu.make_async_copy(out_v.at[rows, :], out_hbm.at[rows, :], out_sem)

    def softmaxes(q, k, keep, pen):
        ps = []
        for j in range(HG):
            cs = slice(j * dh, (j + 1) * dh)
            s = _dot_nt(q[:, cs], k[:, cs]) * scale
            rs = slice(keep.shape[0] - s.shape[0], keep.shape[0])
            s = jnp.where(keep[rs, :] > 0.5, s, pen[rs, :])
            e = jnp.exp(s - jnp.max(s, axis=-1, keepdims=True))
            ps.append((e / jnp.sum(e, axis=-1, keepdims=True)).astype(BF16))
        return ps

    def weigh_values(g, ps, v):
        for j, p in enumerate(ps):
            o = _dot(p, v[:, j * dh:(j + 1) * dh])
            o_buf[g, 0:p.shape[0] // 2, j * dh:(j + 1) * dh] = _pack(o)

    def attention(qkv, keep, pen, fillers):
        fillers = list(fillers)
        ready = [qkv(0), qkv(1)]
        for g in range(n_groups):
            q, k, v = ready[g]
            ps = softmaxes(q, k, keep, pen)
            if g + 2 < n_groups:
                ready.append(qkv(g + 2))
            if fillers:
                fillers.pop(0)()
            weigh_values(g, ps, v)
        for f in fillers:
            f()

    def ffn_up(yn, c):
        cs = slice(c * FC, (c + 1) * FC)
        gate = _dot(yn, _bf16(wg[:, cs]))
        up = _dot(yn, _bf16(wu[:, cs]))
        a_buf[0:yn.shape[0] // 2, cs] = _pack(_gelu(gate) * up)

    def ffn_down(rows, lo, hi):
        return _dot(get(a_buf, 0, rows), _bf16(wd[:, lo:hi]))

    def ffn_fillers(y, parts):
        yn = _layernorm(y).astype(BF16)
        split = d_model // 4

        def down(lo, hi):
            parts.append(y[:, lo:hi] + ffn_down(y.shape[0], lo, hi))

        up = [functools.partial(ffn_up, yn, c) for c in range(n_chunks)]
        return up[:-2] + [lambda: (up[-2](), up[-1]()),
                          lambda: down(0, split),
                          lambda: down(split, d_model)]

    def out_proj(rows, between=lambda: None):
        cut = d_model // 2
        o = jnp.concatenate(
            [_bf16(o_buf[g, 0:rows // 2, :]) for g in range(n_groups)], axis=1)
        left = _dot(o, _bf16(wo[:, 0:cut]))
        between()
        return jnp.concatenate([left, _dot(o, _bf16(wo[:, cut:]))], axis=1)

    def put_mem_one_layer(r, first):
        ri = jax.lax.broadcasted_iota(jnp.int32, (mt, d_model), 0)
        act = (ri < n_mem) if first else (ri >= n_mem)
        put(h_buf, 0, jnp.where(act, r, get(h_buf, 0, mt).astype(F32)))

    def project(h, g):
        return [_dot(h, _bf16(w[g])).astype(BF16) for w in w3]

    def main_step(t, use_pre):
        if use_pre:
            h = jnp.concatenate(
                [get(h_buf, 0, mt), get(h_buf, mt + seg, mt + 2 * seg)], axis=0)
            ps = pl.ds(pl.multiple_of((pre0 + (t - 2) * seg) // 2, 8), seg // 2)

            def qkv(g):
                return [jnp.concatenate([r[0:mt], _bf16(p[g, ps, :]), r[mt:]], axis=0)
                        for r, p in zip(project(h, g), pre)]
        else:
            qkv = functools.partial(project, get(h_buf, 0, mt + 2 * seg))
        z_old = z_buf[...]
        y = y_buf[...]
        if not use_pre:
            put(h_buf, mt, _layernorm(x_seg(jnp.minimum(t + 1, n_seg - 1))))
        t_out = jnp.maximum(t - 3, 0)
        parts = []

        def finish():
            z = jnp.concatenate(parts, axis=1)
            z_buf[...] = z[0:seg]
            put(h_buf, mt + seg, _layernorm(z[0:seg]))
            out_v[seg_rows(t_out), :] = z[seg:2 * seg].astype(BF16)

        attention(qkv, keep_full, pen_full, ffn_fillers(y, parts))
        r = out_proj(mt + 2 * seg, finish)
        put(h_buf, 0, r[0:mt])
        y_buf[0:seg, :] = x_seg(t) + r[mt:mt + seg]
        y_buf[seg:2 * seg, :] = z_old + r[mt + seg:mt + 2 * seg]

        pl.when(t >= 3)(lambda: out_copy(t_out, 1).start())

    scope = jax.named_scope
    with scope("p0_wait_x"):
        x_copies[0].wait()
    w3_start(1, 2 * n_groups)
    m0 = mem_v[...].astype(F32)
    m0 = jnp.concatenate([m0, m0], axis=0)
    put(h_buf, 0, m0)
    put(xpre, 0, m0)
    put(xpre, mt, _layernorm(x_seg(0)))
    put(xpre, mt + seg, _layernorm(x_seg(1))[0:half])
    for s in range(n_pre):
        put(xpre, pre0 + s * seg, _layernorm(x_seg(2 + s)))
    put(h_buf, mt, _layernorm(x_seg(2 + n_pre)))
    y_buf[seg:2 * seg, :] = jnp.zeros((seg, d_model), F32)

    kq = d_model // 2
    nq = n_groups // 2

    def q_group(s, g, chunk=None):
        xs = _bf16(xpre[:, s * kq:(s + 1) * kq])
        for j in range(HG):
            cs = slice(j * dh, (j + 1) * dh)
            if chunk:
                relayout(*chunk, j, j + 1)
            r = _dot(xs, _bf16(wq[g, s * kq // 2:(s + 1) * kq // 2, cs]))
            if s == 0:
                q_acc[g, :, cs] = r
            else:
                q_pre[g, :, cs] = _pack(q_acc[g, :, cs] + r)

    def first_chunk(c):
        w3_wait(c)
        relayout(0, c)

    with scope("p1_project_q"):
        _loop(0, nq, first_chunk)
        _loop(0, nq, lambda g: q_group(0, g), 2)
        _loop(nq, n_groups, lambda g: q_group(0, g, (0, g)), 2, w3_wait)
        w3_start(2 * n_groups, 3 * n_groups)
        _loop(0, n_groups, lambda g: q_group(1, g, (1, g)), 2,
              lambda g: w3_wait(n_groups + g))

    def project_group(m, g, side_work=lambda j: None):
        xs = _bf16(xpre[...])
        for j in range(HG):
            cs = slice(j * dh, (j + 1) * dh)
            side_work(j)
            pre[m][g, :, cs] = _pack(_dot(xs, _bf16(w3[m][g, :, cs])))

    def precomputed(p, g, lo, hi):
        return _bf16(p[g, lo // 2:hi // 2, :])

    def k_group(g):
        project_group(1, g, lambda j: relayout(2, g, j, j + 1))

    def v_group(g):
        ps = softmaxes(precomputed(q_pre, g, 0, mt + seg), precomputed(k_pre, g, 0, mt + seg),
                       keep_one, pen_one)
        project_group(2, g)
        weigh_values(g, ps, precomputed(v_pre, g, 0, mt + seg))

    w_copies[0].start()
    w_copies[1].start()
    with scope("p3_project_k"):
        _loop(0, n_groups, k_group, 1, lambda g: w3_wait(2 * n_groups + g))
    w_copies[2].start()
    w_copies[3].start()
    x_copies[1].start()
    with scope("p4_project_v"):
        _loop(0, n_groups, v_group)

    with scope("p5_seg0"):
        w_copies[0].wait()
        r = out_proj(mt + seg)
        put_mem_one_layer(r[0:mt], True)
        y_buf[0:seg, :] = x_seg(0) + r[mt:]

    with scope("p6_seg1"):
        w_copies[1].wait()
        w_copies[2].wait()
        late = _layernorm(x_seg(1))[half:].astype(BF16)
        hm = jnp.concatenate([get(h_buf, 0, mt), late], axis=0)
        yn = _layernorm(y_buf[0:seg, :]).astype(BF16)
        attention(
            lambda g: [jnp.concatenate(
                [r[0:mt], precomputed(p, g, mt + seg, pre0), r[mt:]], axis=0)
                       for r, p in zip(project(hm, g), pre)],
            keep_one, pen_one, [functools.partial(ffn_up, yn, c) for c in range(n_chunks)])
        r = out_proj(mt + seg)
        put_mem_one_layer(r[0:mt], True)
        z_buf[...] = x_seg(1) + r[mt:]

    with scope("p7_ffn0"):
        w_copies[3].wait()
        z = y_buf[0:seg, :] + ffn_down(seg, 0, d_model)
        y_buf[0:seg, :] = z_buf[...]
        z_buf[...] = z
        put(h_buf, mt + seg, _layernorm(z))

    with scope("p8_main_pre"):
        _loop(2, 2 + n_pre, lambda t: main_step(t, True))
    x_copies[1].wait()
    with scope("p9_main"):
        _loop(2 + n_pre, n_seg, lambda t: main_step(t, False))

    def second_layer_only(t):
        first = t == n_seg
        h = jnp.concatenate(
            [get(h_buf, 0, mt), get(h_buf, mt + seg, mt + 2 * seg)], axis=0)
        z_old = z_buf[...]
        parts = []

        def finish():
            z = jnp.concatenate(parts, axis=1)
            if first:
                z_buf[...] = z[0:seg]
                put(h_buf, mt + seg, _layernorm(z[0:seg]))
            out_v[(t - 3) * seg:(t - 2) * seg, :] = z[z.shape[0] - seg:].astype(BF16)

        lo = 0 if first else mt

        def qkv(g):
            return [_dot(a, _bf16(w[g])).astype(BF16) for a, w in zip((h[lo:], h, h), w3)]

        attention(qkv, keep_two, pen_two,
                  ffn_fillers(y_buf[0 if first else seg:2 * seg, :], parts))
        r = out_proj(mt + seg - lo, finish)
        if first:
            put_mem_one_layer(r[0:mt], False)
        y_buf[seg:2 * seg, :] = z_old + r[mt - lo:]
        out_copy(t - 3, 1).start()

    with scope("pa_e0"):
        second_layer_only(n_seg)
    with scope("pb_e1"):
        second_layer_only(n_seg + 1)
    with scope("pc_e2"):
        y = y_buf[seg:2 * seg, :]
        yn = _layernorm(y).astype(BF16)
        for c in range(n_chunks):
            ffn_up(yn, c)
        z = y + ffn_down(seg, 0, d_model)
        out_v[(n_seg - 1) * seg:n_seg * seg, :] = z.astype(BF16)
        out_copy(n_seg - 1, 1).start()
        pltpu.make_async_copy(out_v, out_hbm, out_sem).wait()


@functools.partial(jax.jit, static_argnames=("A_seg_len",))
def pallas_interleave_layers__memory_aug_recurrent_mem_tr__glu_gated_geglu__prompt_kernel(
    A_x, A_mem0, A_Wq, A_Wk, A_Wv, A_Wo, A_seg_len, B_x, B_w_gate, B_w_up, B_w_down,
):
    del B_x
    _, S, Dm = A_x.shape
    _, M, _ = A_mem0.shape
    _, H, Dh = A_Wq.shape
    Df = B_w_gate.shape[1]
    seg = int(A_seg_len)
    n_seg = S // seg
    mt = 2 * M
    G = H // HG
    gw = HG * Dh
    rows = mt + 2 * seg
    pre_rows = mt + seg + seg // 2 + N_PRE * seg

    kern = functools.partial(
        _kernel, n_seg=n_seg, seg=seg, n_mem=M, n_heads=H, dh=Dh, n_pre=N_PRE)
    any_spec = pl.BlockSpec(memory_space=pl.ANY)
    out = pl.pallas_call(
        kern,
        in_specs=[any_spec, pl.BlockSpec(memory_space=pltpu.VMEM)] + [any_spec] * 7,
        out_specs=any_spec,
        out_shape=jax.ShapeDtypeStruct((S, Dm), A_x.dtype),
        scratch_shapes=[
            pltpu.VMEM((S, Dm), BF16),
            pltpu.VMEM((3 * G, Dm // G * H, Dh), BF16),
            pltpu.VMEM((4, Dm // G * H // 8, Dh), U32),
            pltpu.VMEM((G, Dm // 2, gw), U32),
            pltpu.VMEM((G, Dm // 2, gw), U32),
            pltpu.VMEM((G, Dm // 2, gw), U32),
            pltpu.VMEM((H * Dh // 2, Dm), U32),
            pltpu.VMEM((Dm // 2, Df), U32),
            pltpu.VMEM((Dm // 2, Df), U32),
            pltpu.VMEM((Df // 2, Dm), U32),
            pltpu.VMEM((pre_rows // 2, Dm), U32),
            pltpu.VMEM((G, pre_rows, gw), F32),
            pltpu.VMEM((G, pre_rows // 2, gw), U32),
            pltpu.VMEM((G, pre_rows // 2, gw), U32),
            pltpu.VMEM((G, pre_rows // 2, gw), U32),
            pltpu.VMEM((rows // 2, Dm), U32),
            pltpu.VMEM((G, rows // 2, gw), U32),
            pltpu.VMEM((2 * seg, Dm), F32),
            pltpu.VMEM((seg, Dm), F32),
            pltpu.VMEM((seg, Df), U32),
            pltpu.VMEM((rows, rows), F32),
            pltpu.VMEM((rows, rows), F32),
            pltpu.VMEM((mt + seg, mt + seg), F32),
            pltpu.VMEM((mt + seg, mt + seg), F32),
            pltpu.VMEM((mt + seg, mt + seg), F32),
            pltpu.VMEM((mt + seg, mt + seg), F32),
            pltpu.VMEM((S, Dm), BF16),
            pltpu.SemaphoreType.DMA((2,)),
            pltpu.SemaphoreType.DMA((3 * G,)),
            pltpu.SemaphoreType.DMA((4,)),
            pltpu.SemaphoreType.DMA(()),
        ],
        compiler_params=pltpu.CompilerParams(vmem_limit_bytes=124 * 1024 * 1024),
    )(
        A_x.reshape(S, Dm), A_mem0.reshape(M, Dm),
        A_Wq.reshape(Dm * H, Dh), A_Wk.reshape(Dm * H, Dh), A_Wv.reshape(Dm * H, Dh),
        A_Wo.reshape(H * Dh, Dm), B_w_gate, B_w_up, B_w_down,
    )
    return out.reshape(1, S, Dm)
```

```python
import functools

import jax
import jax.numpy as jnp
import numpy as np
import jax.experimental.pallas as pl
import jax.experimental.pallas.tpu as pltpu

F32 = jnp.float32
BF16 = jnp.bfloat16
U32 = jnp.uint32
LN_EPS = 1e-5
HG = 4
FC = 512
N_PRE = 11


def _layernorm(x):
    m = jnp.mean(x, axis=-1, keepdims=True)
    xc = x - m
    v = jnp.mean(xc * xc, axis=-1, keepdims=True)
    return xc * jax.lax.rsqrt(v + LN_EPS)


def _gelu(x):
    c = float(np.sqrt(2.0 / np.pi))
    return x * (0.5 * (1.0 + jnp.tanh(c * (x + 0.044715 * (x * x * x)))))


def _dot(a, b):
    return jnp.dot(a, b, preferred_element_type=F32)


def _dot_nt(a, b):
    return jax.lax.dot_general(a, b, (((1,), (1,)), ((), ())), preferred_element_type=F32)


def _pack(x):
    return pltpu.bitcast(x.astype(BF16), U32)


def _bf16(words):
    return pltpu.bitcast(words, BF16)


def _loop(lo, hi, fn, unroll=1, first=None):
    assert (hi - lo) % unroll == 0

    def body(i, carry):
        steps = [lo + i * unroll + u for u in range(unroll)]
        for stage in ((first, fn) if first else (fn,)):
            for t in steps:
                stage(t)
        return carry
    jax.lax.fori_loop(0, (hi - lo) // unroll, body, 0)


def _kernel(x_hbm, mem_hbm, wq_hbm, wk_hbm, wv_hbm, wo_hbm, wg_hbm, wu_hbm, wd_hbm,
            out_hbm,
            x_v, mem_v, stage, tmp, wq, wk, wv, wo, wg, wu, wd,
            xpre, q_acc, q_pre, k_pre, v_pre, h_buf, o_buf, y_buf, z_buf, a_buf,
            keep_full, pen_full, keep_one, pen_one, keep_two, pen_two,
            out_v, x_sem, w3_sem, w_sem, out_sem,
            *, n_seg, seg, n_mem, n_heads, dh, n_pre):
    d_model = x_v.shape[1]
    d_ff = wg.shape[1]
    mt = 2 * n_mem
    scale = float(dh) ** -0.5
    half = seg // 2
    pre0 = mt + seg + half
    n_groups = n_heads // HG
    gw = HG * dh
    n_chunks = d_ff // FC
    dc = d_model // n_groups
    crows = dc * n_heads
    pairs = n_heads // 2
    w3 = (wq, wk, wv)
    pre = (q_pre, k_pre, v_pre)

    def get(ref, lo, hi):
        return _bf16(ref[lo // 2:hi // 2, :])

    def put(ref, lo, x):
        ref[lo // 2:(lo + x.shape[0]) // 2, :] = _pack(x)

    x_head = (2 + n_pre + 1) * seg
    x_copies = [
        pltpu.make_async_copy(x_hbm.at[lo:hi, :], x_v.at[lo:hi, :], x_sem.at[i])
        for i, (lo, hi) in enumerate(((0, x_head), (x_head, n_seg * seg)))]
    mem_copy = pltpu.make_async_copy(mem_hbm, mem_v, x_sem.at[2])
    w_copies = [pltpu.make_async_copy(s.bitcast(U32), d, w_sem.at[i]) for i, (s, d) in
                enumerate(((wo_hbm, wo), (wg_hbm, wg), (wu_hbm, wu), (wd_hbm, wd)))]

    def w3_start(lo, hi):
        for i in range(lo, hi):
            m, c = divmod(i, n_groups)
            src = (wq_hbm, wk_hbm, wv_hbm)[m]
            pltpu.make_async_copy(
                src.at[c * crows:(c + 1) * crows, :], stage.at[i], w3_sem.at[i]).start()

    def w3_wait(i):
        pltpu.make_async_copy(stage.at[i], stage.at[i], w3_sem.at[i]).wait()

    mem_copy.start()
    x_copies[0].start()
    w3_start(0, 1)

    stage_words = stage.bitcast(U32)

    def relayout(m, c, q_lo=0, q_hi=4):
        i = m * n_groups + c
        rows = pl.ds(pl.multiple_of(c * (dc // 2), dc // 2), dc // 2)
        for lo in range(q_lo, q_hi):
            tmp[lo] = stage_words[i, pl.ds(lo, dc * pairs // 4, stride=4), :]
            for a in range(pairs // 4):
                even = tmp[lo, pl.ds(a, dc // 2, stride=pairs // 2), :]
                odd = tmp[lo, pl.ds(pairs // 4 + a, dc // 2, stride=pairs // 2), :]
                g, j = divmod(2 * (4 * a + lo), HG)
                w3[m][g, rows, j * dh:(j + 1) * dh] = (even & U32(0xFFFF)) | (odd << 16)
                w3[m][g, rows, (j + 1) * dh:(j + 2) * dh] = (
                    (even >> 16) | (odd & U32(0xFFFF0000)))

    def make_mask(rows, x_layers):
        qi = jax.lax.broadcasted_iota(jnp.int32, (rows, rows), 0)
        ki = jax.lax.broadcasted_iota(jnp.int32, (rows, rows), 1)

        def layer(i):
            lm = jnp.where(i < n_mem, 0, 1)
            return jnp.where(i < mt, lm, jnp.where(i < mt + seg, x_layers[0], x_layers[-1]))

        def pos(i):
            pm = jnp.where(i < n_mem, i, i - n_mem)
            px = jnp.where(i < mt + seg, i - mt, i - mt - seg) + n_mem
            return jnp.where(i < mt, pm, px)

        same = layer(qi) == layer(ki)
        causal = (pos(qi) < n_mem) | (pos(qi) >= pos(ki))
        keep = jnp.where(same & causal, 1.0, 0.0).astype(F32)
        pen = jnp.where(same, -1e9, -jnp.inf).astype(F32)
        return keep, pen

    keep_full[...], pen_full[...] = make_mask(mt + 2 * seg, (0, 1))
    keep_one[...], pen_one[...] = make_mask(mt + seg, (0,))
    keep_two[...], pen_two[...] = make_mask(mt + seg, (1,))

    def seg_rows(t):
        return pl.ds(pl.multiple_of(t * seg, seg), seg)

    def x_seg(t):
        return x_v[seg_rows(t), :].astype(F32)

    def out_copy(t, n):
        rows = pl.ds(pl.multiple_of(t * seg, seg), n * seg)
        return pltpu.make_async_copy(out_v.at[rows, :], out_hbm.at[rows, :], out_sem)

    def softmaxes(q, k, keep, pen):
        ps = []
        for j in range(HG):
            cs = slice(j * dh, (j + 1) * dh)
            s = _dot_nt(q[:, cs], k[:, cs]) * scale
            rs = slice(keep.shape[0] - s.shape[0], keep.shape[0])
            s = jnp.where(keep[rs, :] > 0.5, s, pen[rs, :])
            e = jnp.exp(s - jnp.max(s, axis=-1, keepdims=True))
            ps.append((e / jnp.sum(e, axis=-1, keepdims=True)).astype(BF16))
        return ps

    def weigh_values(g, ps, v):
        for j, p in enumerate(ps):
            o = _dot(p, v[:, j * dh:(j + 1) * dh])
            o_buf[g, 0:p.shape[0] // 2, j * dh:(j + 1) * dh] = _pack(o)

    def attention(qkv, keep, pen, fillers):
        fillers = list(fillers)
        ready = [qkv(0), qkv(1)]
        for g in range(n_groups):
            q, k, v = ready[g]
            ps = softmaxes(q, k, keep, pen)
            if g + 2 < n_groups:
                ready.append(qkv(g + 2))
            if fillers:
                fillers.pop(0)()
            weigh_values(g, ps, v)
        for f in fillers:
            f()

    def ffn_up(yn, c):
        cs = slice(c * FC, (c + 1) * FC)
        gate = _dot(yn, _bf16(wg[:, cs]))
        up = _dot(yn, _bf16(wu[:, cs]))
        a_buf[0:yn.shape[0] // 2, cs] = _pack(_gelu(gate) * up)

    def ffn_down(rows, lo, hi):
        return _dot(get(a_buf, 0, rows), _bf16(wd[:, lo:hi]))

    def ffn_fillers(y, parts):
        yn = _layernorm(y).astype(BF16)
        split = d_model // 4

        def down(lo, hi):
            parts.append(y[:, lo:hi] + ffn_down(y.shape[0], lo, hi))

        up = [functools.partial(ffn_up, yn, c) for c in range(n_chunks)]
        return up[:-2] + [lambda: (up[-2](), up[-1]()),
                          lambda: down(0, split),
                          lambda: down(split, d_model)]

    def out_proj(rows, between=lambda: None):
        cut = d_model // 2
        o = jnp.concatenate(
            [_bf16(o_buf[g, 0:rows // 2, :]) for g in range(n_groups)], axis=1)
        left = _dot(o, _bf16(wo[:, 0:cut]))
        between()
        return jnp.concatenate([left, _dot(o, _bf16(wo[:, cut:]))], axis=1)

    def put_mem_one_layer(r, first):
        ri = jax.lax.broadcasted_iota(jnp.int32, (mt, d_model), 0)
        act = (ri < n_mem) if first else (ri >= n_mem)
        put(h_buf, 0, jnp.where(act, r, get(h_buf, 0, mt).astype(F32)))

    def project(h, g):
        return [_dot(h, _bf16(w[g])).astype(BF16) for w in w3]

    def main_step(t, use_pre, z_next=None):
        if use_pre:
            h = jnp.concatenate(
                [get(h_buf, 0, mt), get(h_buf, mt + seg, mt + 2 * seg)], axis=0)
            ps = pl.ds(pl.multiple_of((pre0 + (t - 2) * seg) // 2, 8), seg // 2)

            def qkv(g):
                return [jnp.concatenate([r[0:mt], _bf16(p[g, ps, :]), r[mt:]], axis=0)
                        for r, p in zip(project(h, g), pre)]
        else:
            qkv = functools.partial(project, get(h_buf, 0, mt + 2 * seg))
        z_old = z_buf[...]
        if not use_pre:
            put(h_buf, mt, _layernorm(x_seg(jnp.minimum(t + 1, n_seg - 1))))
        parts = []

        def finish():
            z1 = z_next
            if z1 is None:
                z = jnp.concatenate(parts, axis=1)
                z1 = z[0:seg]
                out_v[seg_rows(t - 3), :] = z[seg:2 * seg].astype(BF16)
            z_buf[...] = z1
            put(h_buf, mt + seg, _layernorm(z1))

        attention(qkv, keep_full, pen_full,
                  ffn_fillers(y_buf[...], parts) if z_next is None else [])
        r = out_proj(mt + 2 * seg, finish)
        put(h_buf, 0, r[0:mt])
        y_buf[0:seg, :] = x_seg(t) + r[mt:mt + seg]
        y_buf[seg:2 * seg, :] = z_old + r[mt + seg:mt + 2 * seg]
        if z_next is None:
            out_copy(t - 3, 1).start()

    scope = jax.named_scope
    with scope("p0_wait_x"):
        x_copies[0].wait()
        mem_copy.wait()
    w3_start(1, 2 * n_groups)
    m0 = mem_v[...].astype(F32)
    m0 = jnp.concatenate([m0, m0], axis=0)
    put(h_buf, 0, m0)
    put(xpre, 0, m0)
    put(xpre, mt, _layernorm(x_seg(0)))
    put(xpre, mt + seg, _layernorm(x_seg(1))[0:half])
    for s in range(n_pre):
        put(xpre, pre0 + s * seg, _layernorm(x_seg(2 + s)))
    put(h_buf, mt, _layernorm(x_seg(2 + n_pre)))

    kq = d_model // 2
    nq = n_groups // 2

    def q_group(s, g, chunk=None):
        xs = _bf16(xpre[:, s * kq:(s + 1) * kq])
        for j in range(HG):
            cs = slice(j * dh, (j + 1) * dh)
            if chunk:
                relayout(*chunk, j, j + 1)
            r = _dot(xs, _bf16(wq[g, s * kq // 2:(s + 1) * kq // 2, cs]))
            if s == 0:
                q_acc[g, :, cs] = r
            else:
                q_pre[g, :, cs] = _pack(q_acc[g, :, cs] + r)

    def first_chunk(c):
        w3_wait(c)
        relayout(0, c)

    with scope("p1_project_q"):
        _loop(0, nq, first_chunk)
        _loop(0, nq, lambda g: q_group(0, g), 2)
        _loop(nq, n_groups, lambda g: q_group(0, g, (0, g)), 2, w3_wait)
        w3_start(2 * n_groups, 3 * n_groups)
        _loop(0, n_groups, lambda g: q_group(1, g, (1, g)), 2,
              lambda g: w3_wait(n_groups + g))

    def project_group(m, g, side_work=lambda j: None):
        xs = _bf16(xpre[...])
        for j in range(HG):
            cs = slice(j * dh, (j + 1) * dh)
            side_work(j)
            pre[m][g, :, cs] = _pack(_dot(xs, _bf16(w3[m][g, :, cs])))

    def precomputed(p, g, lo, hi):
        return _bf16(p[g, lo // 2:hi // 2, :])

    def k_group(g):
        project_group(1, g, lambda j: relayout(2, g, j, j + 1))

    def v_group(g):
        ps = softmaxes(precomputed(q_pre, g, 0, mt + seg), precomputed(k_pre, g, 0, mt + seg),
                       keep_one, pen_one)
        project_group(2, g)
        weigh_values(g, ps, precomputed(v_pre, g, 0, mt + seg))

    w_copies[0].start()
    w_copies[1].start()
    with scope("p3_project_k"):
        _loop(0, n_groups, k_group, 1, lambda g: w3_wait(2 * n_groups + g))
    w_copies[2].start()
    w_copies[3].start()
    x_copies[1].start()
    with scope("p4_project_v"):
        _loop(0, n_groups, v_group)

    with scope("p5_seg0"):
        w_copies[0].wait()
        r = out_proj(mt + seg)
        put_mem_one_layer(r[0:mt], True)
        y_buf[0:seg, :] = x_seg(0) + r[mt:]

    with scope("p6_seg1"):
        late = _layernorm(x_seg(1))[half:].astype(BF16)
        hm = jnp.concatenate([get(h_buf, 0, mt), late], axis=0)
        attention(
            lambda g: [jnp.concatenate(
                [r[0:mt], precomputed(p, g, mt + seg, pre0), r[mt:]], axis=0)
                       for r, p in zip(project(hm, g), pre)],
            keep_one, pen_one, [])
        r = out_proj(mt + seg)
        put_mem_one_layer(r[0:mt], True)
        y_buf[seg:2 * seg, :] = x_seg(1) + r[mt:]

    with scope("p7_ffn01"):
        w_copies[1].wait()
        w_copies[2].wait()
        y = y_buf[...]
        yn = _layernorm(y).astype(BF16)
        for c in range(n_chunks):
            ffn_up(yn, c)
        w_copies[3].wait()
        z = y + ffn_down(2 * seg, 0, d_model)
        z_buf[...] = z[0:seg]
        put(h_buf, mt + seg, _layernorm(z[0:seg]))
        main_step(2, True, z[seg:2 * seg])

    with scope("p8_main_pre"):
        _loop(3, 2 + n_pre, lambda t: main_step(t, True))
    x_copies[1].wait()
    with scope("p9_main"):
        _loop(2 + n_pre, n_seg, lambda t: main_step(t, False))

    def second_layer_only(t):
        first = t == n_seg
        h = jnp.concatenate(
            [get(h_buf, 0, mt), get(h_buf, mt + seg, mt + 2 * seg)], axis=0)
        z_old = z_buf[...]
        parts = []

        def finish():
            z = jnp.concatenate(parts, axis=1)
            if first:
                z_buf[...] = z[0:seg]
                put(h_buf, mt + seg, _layernorm(z[0:seg]))
            out_v[(t - 3) * seg:(t - 2) * seg, :] = z[z.shape[0] - seg:].astype(BF16)

        lo = 0 if first else mt

        def qkv(g):
            return [_dot(a, _bf16(w[g])).astype(BF16) for a, w in zip((h[lo:], h, h), w3)]

        attention(qkv, keep_two, pen_two,
                  ffn_fillers(y_buf[0 if first else seg:2 * seg, :], parts))
        r = out_proj(mt + seg - lo, finish)
        if first:
            put_mem_one_layer(r[0:mt], False)
        y_buf[seg:2 * seg, :] = z_old + r[mt - lo:]
        out_copy(t - 3, 1).start()

    with scope("pa_e0"):
        second_layer_only(n_seg)
    with scope("pb_e1"):
        second_layer_only(n_seg + 1)
    with scope("pc_e2"):
        y = y_buf[seg:2 * seg, :]
        yn = _layernorm(y).astype(BF16)
        for c in range(n_chunks):
            ffn_up(yn, c)
        z = y + ffn_down(seg, 0, d_model)
        out_v[(n_seg - 1) * seg:n_seg * seg, :] = z.astype(BF16)
        out_copy(n_seg - 1, 1).start()
        pltpu.make_async_copy(out_v, out_hbm, out_sem).wait()


@functools.partial(jax.jit, static_argnames=("A_seg_len",))
def pallas_interleave_layers__memory_aug_recurrent_mem_tr__glu_gated_geglu__prompt_kernel(
    A_x, A_mem0, A_Wq, A_Wk, A_Wv, A_Wo, A_seg_len, B_x, B_w_gate, B_w_up, B_w_down,
):
    del B_x
    _, S, Dm = A_x.shape
    _, M, _ = A_mem0.shape
    _, H, Dh = A_Wq.shape
    Df = B_w_gate.shape[1]
    seg = int(A_seg_len)
    n_seg = S // seg
    mt = 2 * M
    G = H // HG
    gw = HG * Dh
    rows = mt + 2 * seg
    pre_rows = mt + seg + seg // 2 + N_PRE * seg

    kern = functools.partial(
        _kernel, n_seg=n_seg, seg=seg, n_mem=M, n_heads=H, dh=Dh, n_pre=N_PRE)
    any_spec = pl.BlockSpec(memory_space=pl.ANY)
    out = pl.pallas_call(
        kern,
        in_specs=[any_spec] * 9,
        out_specs=any_spec,
        out_shape=jax.ShapeDtypeStruct((S, Dm), A_x.dtype),
        scratch_shapes=[
            pltpu.VMEM((S, Dm), BF16),
            pltpu.VMEM((M, Dm), BF16),
            pltpu.VMEM((3 * G, Dm // G * H, Dh), BF16),
            pltpu.VMEM((4, Dm // G * H // 8, Dh), U32),
            pltpu.VMEM((G, Dm // 2, gw), U32),
            pltpu.VMEM((G, Dm // 2, gw), U32),
            pltpu.VMEM((G, Dm // 2, gw), U32),
            pltpu.VMEM((H * Dh // 2, Dm), U32),
            pltpu.VMEM((Dm // 2, Df), U32),
            pltpu.VMEM((Dm // 2, Df), U32),
            pltpu.VMEM((Df // 2, Dm), U32),
            pltpu.VMEM((pre_rows // 2, Dm), U32),
            pltpu.VMEM((G, pre_rows, gw), F32),
            pltpu.VMEM((G, pre_rows // 2, gw), U32),
            pltpu.VMEM((G, pre_rows // 2, gw), U32),
            pltpu.VMEM((G, pre_rows // 2, gw), U32),
            pltpu.VMEM((rows // 2, Dm), U32),
            pltpu.VMEM((G, rows // 2, gw), U32),
            pltpu.VMEM((2 * seg, Dm), F32),
            pltpu.VMEM((seg, Dm), F32),
            pltpu.VMEM((seg, Df), U32),
            pltpu.VMEM((rows, rows), F32),
            pltpu.VMEM((rows, rows), F32),
            pltpu.VMEM((mt + seg, mt + seg), F32),
            pltpu.VMEM((mt + seg, mt + seg), F32),
            pltpu.VMEM((mt + seg, mt + seg), F32),
            pltpu.VMEM((mt + seg, mt + seg), F32),
            pltpu.VMEM((S, Dm), BF16),
            pltpu.SemaphoreType.DMA((3,)),
            pltpu.SemaphoreType.DMA((3 * G,)),
            pltpu.SemaphoreType.DMA((4,)),
            pltpu.SemaphoreType.DMA(()),
        ],
        compiler_params=pltpu.CompilerParams(vmem_limit_bytes=124 * 1024 * 1024),
    )(
        A_x.reshape(S, Dm), A_mem0.reshape(M, Dm),
        A_Wq.reshape(Dm * H, Dh), A_Wk.reshape(Dm * H, Dh), A_Wv.reshape(Dm * H, Dh),
        A_Wo.reshape(H * Dh, Dm), B_w_gate, B_w_up, B_w_down,
    )
    return out.reshape(1, S, Dm)
```

```python
import functools

import jax
import jax.numpy as jnp
import numpy as np
import jax.experimental.pallas as pl
import jax.experimental.pallas.tpu as pltpu

F32 = jnp.float32
BF16 = jnp.bfloat16
U32 = jnp.uint32
LN_EPS = 1e-5
HG = 4
FC = 512
N_PRE = 10


def _layernorm(x):
    m = jnp.mean(x, axis=-1, keepdims=True)
    xc = x - m
    v = jnp.mean(xc * xc, axis=-1, keepdims=True)
    return xc * jax.lax.rsqrt(v + LN_EPS)


def _gelu(x):
    c = float(np.sqrt(2.0 / np.pi))
    return x * (0.5 * (1.0 + jnp.tanh(c * (x + 0.044715 * (x * x * x)))))


def _dot(a, b):
    return jnp.dot(a, b, preferred_element_type=F32)


def _dot_nt(a, b):
    return jax.lax.dot_general(a, b, (((1,), (1,)), ((), ())), preferred_element_type=F32)


def _pack(x):
    return pltpu.bitcast(x.astype(BF16), U32)


def _bf16(words):
    return pltpu.bitcast(words, BF16)


def _loop(lo, hi, fn, unroll=1, first=None):
    assert (hi - lo) % unroll == 0

    def body(i, carry):
        steps = [lo + i * unroll + u for u in range(unroll)]
        for stage in ((first, fn) if first else (fn,)):
            for t in steps:
                stage(t)
        return carry
    jax.lax.fori_loop(0, (hi - lo) // unroll, body, 0)


def _kernel(x_hbm, mem_hbm, wq_hbm, wk_hbm, wv_hbm, wo_hbm, wg_hbm, wu_hbm, wd_hbm,
            out_hbm,
            x_v, mem_v, stage, tmp, wq, wk, wv, wo, wg, wu, wd,
            xpre, q_acc, q_pre, k_pre, v_pre, h_buf, o_buf, y_buf, z_buf, a_buf,
            keep_full, pen_full, keep_one, pen_one, keep_two, pen_two,
            out_v, x_sem, w3_sem, w_sem, out_sem,
            *, n_seg, seg, n_mem, n_heads, dh, n_pre):
    d_model = x_v.shape[1]
    d_ff = wg.shape[1]
    mt = 2 * n_mem
    scale = float(dh) ** -0.5
    half = seg // 2
    pre0 = mt + seg + half
    n_groups = n_heads // HG
    gw = HG * dh
    n_chunks = d_ff // FC
    dc = d_model // n_groups
    crows = dc * n_heads
    pairs = n_heads // 2
    w3 = (wq, wk, wv)
    pre = (q_pre, k_pre, v_pre)

    def get(ref, lo, hi):
        return _bf16(ref[lo // 2:hi // 2, :])

    def put(ref, lo, x):
        ref[lo // 2:(lo + x.shape[0]) // 2, :] = _pack(x)

    x_head = (2 + n_pre + 1) * seg
    x_copies = [
        pltpu.make_async_copy(x_hbm.at[lo:hi, :], x_v.at[lo:hi, :], x_sem.at[i])
        for i, (lo, hi) in enumerate(((0, x_head), (x_head, n_seg * seg)))]
    mem_copy = pltpu.make_async_copy(mem_hbm, mem_v, x_sem.at[2])
    w_copies = [pltpu.make_async_copy(s.bitcast(U32), d, w_sem.at[i]) for i, (s, d) in
                enumerate(((wo_hbm, wo), (wg_hbm, wg), (wu_hbm, wu), (wd_hbm, wd)))]

    def w3_start(lo, hi):
        for i in range(lo, hi):
            m, c = divmod(i, n_groups)
            src = (wq_hbm, wk_hbm, wv_hbm)[m]
            pltpu.make_async_copy(
                src.at[c * crows:(c + 1) * crows, :], stage.at[i], w3_sem.at[i]).start()

    def w3_wait(i):
        pltpu.make_async_copy(stage.at[i], stage.at[i], w3_sem.at[i]).wait()

    mem_copy.start()
    x_copies[0].start()
    w3_start(0, 1)

    stage_words = stage.bitcast(U32)

    def relayout(m, c, q_lo=0, q_hi=4):
        i = m * n_groups + c
        rows = pl.ds(pl.multiple_of(c * (dc // 2), dc // 2), dc // 2)
        for lo in range(q_lo, q_hi):
            tmp[lo] = stage_words[i, pl.ds(lo, dc * pairs // 4, stride=4), :]
            for a in range(pairs // 4):
                even = tmp[lo, pl.ds(a, dc // 2, stride=pairs // 2), :]
                odd = tmp[lo, pl.ds(pairs // 4 + a, dc // 2, stride=pairs // 2), :]
                g, j = divmod(2 * (4 * a + lo), HG)
                w3[m][g, rows, j * dh:(j + 1) * dh] = (even & U32(0xFFFF)) | (odd << 16)
                w3[m][g, rows, (j + 1) * dh:(j + 2) * dh] = (
                    (even >> 16) | (odd & U32(0xFFFF0000)))

    def make_mask(rows, x_layers):
        qi = jax.lax.broadcasted_iota(jnp.int32, (rows, rows), 0)
        ki = jax.lax.broadcasted_iota(jnp.int32, (rows, rows), 1)

        def layer(i):
            lm = jnp.where(i < n_mem, 0, 1)
            return jnp.where(i < mt, lm, jnp.where(i < mt + seg, x_layers[0], x_layers[-1]))

        def pos(i):
            pm = jnp.where(i < n_mem, i, i - n_mem)
            px = jnp.where(i < mt + seg, i - mt, i - mt - seg) + n_mem
            return jnp.where(i < mt, pm, px)

        same = layer(qi) == layer(ki)
        causal = (pos(qi) < n_mem) | (pos(qi) >= pos(ki))
        keep = jnp.where(same & causal, 1.0, 0.0).astype(F32)
        pen = jnp.where(same, -1e9, -jnp.inf).astype(F32)
        return keep, pen

    keep_full[...], pen_full[...] = make_mask(mt + 2 * seg, (0, 1))
    keep_one[...], pen_one[...] = make_mask(mt + seg, (0,))
    keep_two[...], pen_two[...] = make_mask(mt + seg, (1,))

    def seg_rows(t):
        return pl.ds(pl.multiple_of(t * seg, seg), seg)

    def x_seg(t):
        return x_v[seg_rows(t), :].astype(F32)

    def out_copy(t, n):
        rows = pl.ds(pl.multiple_of(t * seg, seg), n * seg)
        return pltpu.make_async_copy(out_v.at[rows, :], out_hbm.at[rows, :], out_sem)

    def softmaxes(q, k, keep, pen):
        ps = []
        for j in range(HG):
            cs = slice(j * dh, (j + 1) * dh)
            s = _dot_nt(q[:, cs], k[:, cs]) * scale
            rs = slice(keep.shape[0] - s.shape[0], keep.shape[0])
            s = jnp.where(keep[rs, :] > 0.5, s, pen[rs, :])
            e = jnp.exp(s - jnp.max(s, axis=-1, keepdims=True))
            ps.append((e / jnp.sum(e, axis=-1, keepdims=True)).astype(BF16))
        return ps

    def weigh_values(g, ps, v):
        for j, p in enumerate(ps):
            o = _dot(p, v[:, j * dh:(j + 1) * dh])
            o_buf[g, 0:p.shape[0] // 2, j * dh:(j + 1) * dh] = _pack(o)

    def attention(qkv, keep, pen, fillers):
        fillers = list(fillers)
        ready = [qkv(0), qkv(1)]
        for g in range(n_groups):
            q, k, v = ready[g]
            ps = softmaxes(q, k, keep, pen)
            if g + 2 < n_groups:
                ready.append(qkv(g + 2))
            if fillers:
                fillers.pop(0)()
            weigh_values(g, ps, v)
        for f in fillers:
            f()

    def ffn_up(yn, c):
        cs = slice(c * FC, (c + 1) * FC)
        gate = _dot(yn, _bf16(wg[:, cs]))
        up = _dot(yn, _bf16(wu[:, cs]))
        a_buf[0:yn.shape[0] // 2, cs] = _pack(_gelu(gate) * up)

    def ffn_down(rows, lo, hi):
        return _dot(get(a_buf, 0, rows), _bf16(wd[:, lo:hi]))

    def ffn_fillers(y, parts):
        yn = _layernorm(y).astype(BF16)
        split = d_model // 4

        def down(lo, hi):
            parts.append(y[:, lo:hi] + ffn_down(y.shape[0], lo, hi))

        up = [functools.partial(ffn_up, yn, c) for c in range(n_chunks)]
        return up[:-2] + [lambda: (up[-2](), up[-1]()),
                          lambda: down(0, split),
                          lambda: down(split, d_model)]

    def out_proj(rows, between=lambda: None):
        cut = d_model // 2
        o = jnp.concatenate(
            [_bf16(o_buf[g, 0:rows // 2, :]) for g in range(n_groups)], axis=1)
        left = _dot(o, _bf16(wo[:, 0:cut]))
        between()
        return jnp.concatenate([left, _dot(o, _bf16(wo[:, cut:]))], axis=1)

    def put_mem_one_layer(r, first):
        ri = jax.lax.broadcasted_iota(jnp.int32, (mt, d_model), 0)
        act = (ri < n_mem) if first else (ri >= n_mem)
        put(h_buf, 0, jnp.where(act, r, get(h_buf, 0, mt).astype(F32)))

    def project(h, g):
        return [_dot(h, _bf16(w[g])).astype(BF16) for w in w3]

    def main_step(t, use_pre, z_next=None):
        if use_pre:
            h = jnp.concatenate(
                [get(h_buf, 0, mt), get(h_buf, mt + seg, mt + 2 * seg)], axis=0)
            ps = pl.ds(pl.multiple_of((pre0 + (t - 2) * seg) // 2, 8), seg // 2)

            def qkv(g):
                return [jnp.concatenate([r[0:mt], _bf16(p[g, ps, :]), r[mt:]], axis=0)
                        for r, p in zip(project(h, g), pre)]
        else:
            qkv = functools.partial(project, get(h_buf, 0, mt + 2 * seg))
        z_old = z_buf[...]
        if not use_pre:
            put(h_buf, mt, _layernorm(x_seg(jnp.minimum(t + 1, n_seg - 1))))
        parts = []

        def finish():
            z1 = z_next
            if z1 is None:
                z = jnp.concatenate(parts, axis=1)
                z1 = z[0:seg]
                out_v[seg_rows(t - 3), :] = z[seg:2 * seg].astype(BF16)
            z_buf[...] = z1
            put(h_buf, mt + seg, _layernorm(z1))

        attention(qkv, keep_full, pen_full,
                  ffn_fillers(y_buf[...], parts) if z_next is None else [])
        r = out_proj(mt + 2 * seg, finish)
        put(h_buf, 0, r[0:mt])
        y_buf[0:seg, :] = x_seg(t) + r[mt:mt + seg]
        y_buf[seg:2 * seg, :] = z_old + r[mt + seg:mt + 2 * seg]
        if z_next is None:
            out_copy(t - 3, 1).start()

    x_copies[0].wait()
    mem_copy.wait()
    w3_start(1, 2 * n_groups)
    m0 = mem_v[...].astype(F32)
    m0 = jnp.concatenate([m0, m0], axis=0)
    put(h_buf, 0, m0)
    put(xpre, 0, m0)
    put(xpre, mt, _layernorm(x_seg(0)))
    put(xpre, mt + seg, _layernorm(x_seg(1))[0:half])
    for s in range(n_pre):
        put(xpre, pre0 + s * seg, _layernorm(x_seg(2 + s)))
    put(h_buf, mt, _layernorm(x_seg(2 + n_pre)))

    kq = d_model // 2
    nq = n_groups // 2

    def q_group(s, g, chunk=None):
        xs = _bf16(xpre[:, s * kq:(s + 1) * kq])
        for j in range(HG):
            cs = slice(j * dh, (j + 1) * dh)
            if chunk:
                relayout(*chunk, j, j + 1)
            r = _dot(xs, _bf16(wq[g, s * kq // 2:(s + 1) * kq // 2, cs]))
            if s == 0:
                q_acc[g, :, cs] = r
            else:
                q_pre[g, :, cs] = _pack(q_acc[g, :, cs] + r)

    def first_chunk(c):
        w3_wait(c)
        relayout(0, c)

    _loop(0, nq, first_chunk)
    _loop(0, nq, lambda g: q_group(0, g), 2)
    _loop(nq, n_groups, lambda g: q_group(0, g, (0, g)), 2, w3_wait)
    w3_start(2 * n_groups, 3 * n_groups)
    _loop(0, n_groups, lambda g: q_group(1, g, (1, g)), 2,
          lambda g: w3_wait(n_groups + g))

    def project_group(m, g, side_work=lambda j: None):
        xs = _bf16(xpre[...])
        for j in range(HG):
            cs = slice(j * dh, (j + 1) * dh)
            side_work(j)
            pre[m][g, :, cs] = _pack(_dot(xs, _bf16(w3[m][g, :, cs])))

    def precomputed(p, g, lo, hi):
        return _bf16(p[g, lo // 2:hi // 2, :])

    def k_group(g):
        project_group(1, g, lambda j: relayout(2, g, j, j + 1))

    def v_group(g):
        ps = softmaxes(precomputed(q_pre, g, 0, mt + seg), precomputed(k_pre, g, 0, mt + seg),
                       keep_one, pen_one)
        project_group(2, g)
        weigh_values(g, ps, precomputed(v_pre, g, 0, mt + seg))

    w_copies[0].start()
    w_copies[1].start()
    _loop(0, n_groups, k_group, 1, lambda g: w3_wait(2 * n_groups + g))
    w_copies[2].start()
    w_copies[3].start()
    x_copies[1].start()
    _loop(0, n_groups, v_group, 2)

    w_copies[0].wait()
    r = out_proj(mt + seg)
    put_mem_one_layer(r[0:mt], True)
    y_buf[0:seg, :] = x_seg(0) + r[mt:]

    late = _layernorm(x_seg(1))[half:].astype(BF16)
    hm = jnp.concatenate([get(h_buf, 0, mt), late], axis=0)
    attention(
        lambda g: [jnp.concatenate(
            [r[0:mt], precomputed(p, g, mt + seg, pre0), r[mt:]], axis=0)
                   for r, p in zip(project(hm, g), pre)],
        keep_one, pen_one, [])
    r = out_proj(mt + seg)
    put_mem_one_layer(r[0:mt], True)
    y_buf[seg:2 * seg, :] = x_seg(1) + r[mt:]

    w_copies[1].wait()
    w_copies[2].wait()
    y = y_buf[...]
    yn = _layernorm(y).astype(BF16)
    for c in range(n_chunks):
        ffn_up(yn, c)
    w_copies[3].wait()
    z = y + ffn_down(2 * seg, 0, d_model)
    z_buf[...] = z[0:seg]
    put(h_buf, mt + seg, _layernorm(z[0:seg]))
    main_step(2, True, z[seg:2 * seg])

    _loop(3, 2 + n_pre, lambda t: main_step(t, True))
    x_copies[1].wait()
    _loop(2 + n_pre, n_seg, lambda t: main_step(t, False))

    def second_layer_only(t):
        first = t == n_seg
        h = jnp.concatenate(
            [get(h_buf, 0, mt), get(h_buf, mt + seg, mt + 2 * seg)], axis=0)
        z_old = z_buf[...]
        parts = []

        def finish():
            z = jnp.concatenate(parts, axis=1)
            if first:
                z_buf[...] = z[0:seg]
                put(h_buf, mt + seg, _layernorm(z[0:seg]))
            out_v[(t - 3) * seg:(t - 2) * seg, :] = z[z.shape[0] - seg:].astype(BF16)

        lo = 0 if first else mt

        def qkv(g):
            return [_dot(a, _bf16(w[g])).astype(BF16) for a, w in zip((h[lo:], h, h), w3)]

        attention(qkv, keep_two, pen_two,
                  ffn_fillers(y_buf[0 if first else seg:2 * seg, :], parts))
        r = out_proj(mt + seg - lo, finish)
        if first:
            put_mem_one_layer(r[0:mt], False)
        y_buf[seg:2 * seg, :] = z_old + r[mt - lo:]
        out_copy(t - 3, 1).start()

    second_layer_only(n_seg)
    second_layer_only(n_seg + 1)
    y = y_buf[seg:2 * seg, :]
    yn = _layernorm(y).astype(BF16)
    for c in range(n_chunks):
        ffn_up(yn, c)
    z = y + ffn_down(seg, 0, d_model)
    out_v[(n_seg - 1) * seg:n_seg * seg, :] = z.astype(BF16)
    out_copy(n_seg - 1, 1).start()
    pltpu.make_async_copy(out_v, out_hbm, out_sem).wait()


@functools.partial(jax.jit, static_argnames=("A_seg_len",))
def pallas_interleave_layers__memory_aug_recurrent_mem_tr__glu_gated_geglu__prompt_kernel(
    A_x, A_mem0, A_Wq, A_Wk, A_Wv, A_Wo, A_seg_len, B_x, B_w_gate, B_w_up, B_w_down,
):
    del B_x
    _, S, Dm = A_x.shape
    _, M, _ = A_mem0.shape
    _, H, Dh = A_Wq.shape
    Df = B_w_gate.shape[1]
    seg = int(A_seg_len)
    n_seg = S // seg
    mt = 2 * M
    G = H // HG
    gw = HG * Dh
    rows = mt + 2 * seg
    pre_rows = mt + seg + seg // 2 + N_PRE * seg

    kern = functools.partial(
        _kernel, n_seg=n_seg, seg=seg, n_mem=M, n_heads=H, dh=Dh, n_pre=N_PRE)
    any_spec = pl.BlockSpec(memory_space=pl.ANY)
    out = pl.pallas_call(
        kern,
        in_specs=[any_spec] * 9,
        out_specs=any_spec,
        out_shape=jax.ShapeDtypeStruct((S, Dm), A_x.dtype),
        scratch_shapes=[
            pltpu.VMEM((S, Dm), BF16),
            pltpu.VMEM((M, Dm), BF16),
            pltpu.VMEM((3 * G, Dm // G * H, Dh), BF16),
            pltpu.VMEM((4, Dm // G * H // 8, Dh), U32),
            pltpu.VMEM((G, Dm // 2, gw), U32),
            pltpu.VMEM((G, Dm // 2, gw), U32),
            pltpu.VMEM((G, Dm // 2, gw), U32),
            pltpu.VMEM((H * Dh // 2, Dm), U32),
            pltpu.VMEM((Dm // 2, Df), U32),
            pltpu.VMEM((Dm // 2, Df), U32),
            pltpu.VMEM((Df // 2, Dm), U32),
            pltpu.VMEM((pre_rows // 2, Dm), U32),
            pltpu.VMEM((G, pre_rows, gw), F32),
            pltpu.VMEM((G, pre_rows // 2, gw), U32),
            pltpu.VMEM((G, pre_rows // 2, gw), U32),
            pltpu.VMEM((G, pre_rows // 2, gw), U32),
            pltpu.VMEM((rows // 2, Dm), U32),
            pltpu.VMEM((G, rows // 2, gw), U32),
            pltpu.VMEM((2 * seg, Dm), F32),
            pltpu.VMEM((seg, Dm), F32),
            pltpu.VMEM((seg, Df), U32),
            pltpu.VMEM((rows, rows), F32),
            pltpu.VMEM((rows, rows), F32),
            pltpu.VMEM((mt + seg, mt + seg), F32),
            pltpu.VMEM((mt + seg, mt + seg), F32),
            pltpu.VMEM((mt + seg, mt + seg), F32),
            pltpu.VMEM((mt + seg, mt + seg), F32),
            pltpu.VMEM((S, Dm), BF16),
            pltpu.SemaphoreType.DMA((3,)),
            pltpu.SemaphoreType.DMA((3 * G,)),
            pltpu.SemaphoreType.DMA((4,)),
            pltpu.SemaphoreType.DMA(()),
        ],
        compiler_params=pltpu.CompilerParams(vmem_limit_bytes=124 * 1024 * 1024),
    )(
        A_x.reshape(S, Dm), A_mem0.reshape(M, Dm),
        A_Wq.reshape(Dm * H, Dh), A_Wk.reshape(Dm * H, Dh), A_Wv.reshape(Dm * H, Dh),
        A_Wo.reshape(H * Dh, Dm), B_w_gate, B_w_up, B_w_down,
    )
    return out.reshape(1, S, Dm)
```

```python
import functools

import jax
import jax.numpy as jnp
import numpy as np
import jax.experimental.pallas as pl
import jax.experimental.pallas.tpu as pltpu

F32 = jnp.float32
BF16 = jnp.bfloat16
U32 = jnp.uint32
LN_EPS = 1e-5
HG = 4
FC = 512
N_PRE = 12


def _layernorm(x):
    m = jnp.mean(x, axis=-1, keepdims=True)
    xc = x - m
    v = jnp.mean(xc * xc, axis=-1, keepdims=True)
    return xc * jax.lax.rsqrt(v + LN_EPS)


def _gelu(x):
    c = float(np.sqrt(2.0 / np.pi))
    return x * (0.5 * (1.0 + jnp.tanh(c * (x + 0.044715 * (x * x * x)))))


def _dot(a, b):
    return jnp.dot(a, b, preferred_element_type=F32)


def _dot_nt(a, b):
    return jax.lax.dot_general(a, b, (((1,), (1,)), ((), ())), preferred_element_type=F32)


def _pack(x):
    return pltpu.bitcast(x.astype(BF16), U32)


def _bf16(words):
    return pltpu.bitcast(words, BF16)


def _loop(lo, hi, fn, unroll=1, first=None):
    assert (hi - lo) % unroll == 0

    def body(i, carry):
        steps = [lo + i * unroll + u for u in range(unroll)]
        for stage in ((first, fn) if first else (fn,)):
            for t in steps:
                stage(t)
        return carry
    jax.lax.fori_loop(0, (hi - lo) // unroll, body, 0)


def _kernel(x_hbm, mem_hbm, wq_hbm, wk_hbm, wv_hbm, wo_hbm, wg_hbm, wu_hbm, wd_hbm,
            out_hbm,
            x_v, mem_v, stage, tmp, wq, wk, wv, wo, wg, wu, wd,
            xpre, q_acc, q_pre, k_pre, v_pre, h_buf, o_buf, y_buf, z_buf, a_buf,
            keep_full, pen_full, keep_one, pen_one, keep_two, pen_two,
            out_v, x_sem, w3_sem, w_sem, out_sem,
            *, n_seg, seg, n_mem, n_heads, dh, n_pre):
    d_model = x_v.shape[1]
    d_ff = wg.shape[1]
    mt = 2 * n_mem
    scale = float(dh) ** -0.5
    half = seg // 2
    pre0 = mt + seg + half
    n_groups = n_heads // HG
    gw = HG * dh
    n_chunks = d_ff // FC
    dc = d_model // n_groups
    crows = dc * n_heads
    pairs = n_heads // 2
    w3 = (wq, wk, wv)
    pre = (q_pre, k_pre, v_pre)

    def get(ref, lo, hi):
        return _bf16(ref[lo // 2:hi // 2, :])

    def put(ref, lo, x):
        ref[lo // 2:(lo + x.shape[0]) // 2, :] = _pack(x)

    x_head = (2 + n_pre + 1) * seg
    x_copies = [
        pltpu.make_async_copy(x_hbm.at[lo:hi, :], x_v.at[lo:hi, :], x_sem.at[i])
        for i, (lo, hi) in enumerate(((0, x_head), (x_head, n_seg * seg)))]
    mem_copy = pltpu.make_async_copy(mem_hbm, mem_v, x_sem.at[2])
    w_copies = [pltpu.make_async_copy(s.bitcast(U32), d, w_sem.at[i]) for i, (s, d) in
                enumerate(((wo_hbm, wo), (wg_hbm, wg), (wu_hbm, wu), (wd_hbm, wd)))]

    def w3_start(lo, hi):
        for i in range(lo, hi):
            m, c = divmod(i, n_groups)
            src = (wq_hbm, wk_hbm, wv_hbm)[m]
            pltpu.make_async_copy(
                src.at[c * crows:(c + 1) * crows, :], stage.at[i], w3_sem.at[i]).start()

    def w3_wait(i):
        pltpu.make_async_copy(stage.at[i], stage.at[i], w3_sem.at[i]).wait()

    mem_copy.start()
    x_copies[0].start()
    w3_start(0, 1)

    stage_words = stage.bitcast(U32)

    def relayout(m, c, q_lo=0, q_hi=4):
        i = m * n_groups + c
        rows = pl.ds(pl.multiple_of(c * (dc // 2), dc // 2), dc // 2)
        for lo in range(q_lo, q_hi):
            tmp[lo] = stage_words[i, pl.ds(lo, dc * pairs // 4, stride=4), :]
            for a in range(pairs // 4):
                even = tmp[lo, pl.ds(a, dc // 2, stride=pairs // 2), :]
                odd = tmp[lo, pl.ds(pairs // 4 + a, dc // 2, stride=pairs // 2), :]
                g, j = divmod(2 * (4 * a + lo), HG)
                w3[m][g, rows, j * dh:(j + 1) * dh] = (even & np.uint32(0xFFFF)) | (odd << 16)
                w3[m][g, rows, (j + 1) * dh:(j + 2) * dh] = (
                    (even >> 16) | (odd & np.uint32(0xFFFF0000)))

    def make_mask(rows, x_layers):
        qi = jax.lax.broadcasted_iota(jnp.int32, (rows, rows), 0)
        ki = jax.lax.broadcasted_iota(jnp.int32, (rows, rows), 1)

        def layer(i):
            lm = jnp.where(i < n_mem, 0, 1)
            return jnp.where(i < mt, lm, jnp.where(i < mt + seg, x_layers[0], x_layers[-1]))

        def pos(i):
            pm = jnp.where(i < n_mem, i, i - n_mem)
            px = jnp.where(i < mt + seg, i - mt, i - mt - seg) + n_mem
            return jnp.where(i < mt, pm, px)

        same = layer(qi) == layer(ki)
        causal = (pos(qi) < n_mem) | (pos(qi) >= pos(ki))
        keep = jnp.where(same & causal, 1.0, 0.0).astype(F32)
        pen = jnp.where(same, -1e9, -jnp.inf).astype(F32)
        return keep, pen

    keep_full[...], pen_full[...] = make_mask(mt + 2 * seg, (0, 1))
    keep_one[...], pen_one[...] = make_mask(mt + seg, (0,))
    keep_two[...], pen_two[...] = make_mask(mt + seg, (1,))

    def seg_rows(t):
        return pl.ds(pl.multiple_of(t * seg, seg), seg)

    def x_seg(t):
        return x_v[seg_rows(t), :].astype(F32)

    def out_copy(t, n):
        rows = pl.ds(pl.multiple_of(t * seg, seg), n * seg)
        return pltpu.make_async_copy(out_v.at[rows, :], out_hbm.at[rows, :], out_sem)

    def softmaxes(q, k, keep, pen):
        ps = []
        for j in range(HG):
            cs = slice(j * dh, (j + 1) * dh)
            s = _dot_nt(q[:, cs], k[:, cs]) * scale
            rs = slice(keep.shape[0] - s.shape[0], keep.shape[0])
            s = jnp.where(keep[rs, :] > 0.5, s, pen[rs, :])
            e = jnp.exp(s - jnp.max(s, axis=-1, keepdims=True))
            ps.append((e / jnp.sum(e, axis=-1, keepdims=True)).astype(BF16))
        return ps

    def weigh_values(g, ps, v):
        for j, p in enumerate(ps):
            o = _dot(p, v[:, j * dh:(j + 1) * dh])
            o_buf[g, 0:p.shape[0] // 2, j * dh:(j + 1) * dh] = _pack(o)

    def attention(qkv, keep, pen, fillers):
        fillers = list(fillers)
        ready = [qkv(0), qkv(1)]
        for g in range(n_groups):
            q, k, v = ready[g]
            ps = softmaxes(q, k, keep, pen)
            if g + 2 < n_groups:
                ready.append(qkv(g + 2))
            if fillers:
                fillers.pop(0)()
            weigh_values(g, ps, v)
        for f in fillers:
            f()

    def ffn_up(yn, c):
        cs = slice(c * FC, (c + 1) * FC)
        gate = _dot(yn, _bf16(wg[:, cs]))
        up = _dot(yn, _bf16(wu[:, cs]))
        a_buf[0:yn.shape[0] // 2, cs] = _pack(_gelu(gate) * up)

    def ffn_down(rows, lo, hi):
        return _dot(get(a_buf, 0, rows), _bf16(wd[:, lo:hi]))

    def ffn_fillers(y, parts):
        yn = _layernorm(y).astype(BF16)
        split = d_model // 4

        def down(lo, hi):
            parts.append(y[:, lo:hi] + ffn_down(y.shape[0], lo, hi))

        up = [functools.partial(ffn_up, yn, c) for c in range(n_chunks)]
        return up[:-2] + [lambda: (up[-2](), up[-1]()),
                          lambda: down(0, split),
                          lambda: down(split, d_model)]

    def out_proj(rows, between=lambda: None):
        cut = d_model // 2
        o = jnp.concatenate(
            [_bf16(o_buf[g, 0:rows // 2, :]) for g in range(n_groups)], axis=1)
        left = _dot(o, _bf16(wo[:, 0:cut]))
        between()
        return jnp.concatenate([left, _dot(o, _bf16(wo[:, cut:]))], axis=1)

    def attention_and_out_proj(qkv, keep, pen):
        rows = keep.shape[0]
        sums = []

        def groups(lo, hi):
            o = jnp.concatenate(
                [_bf16(o_buf[g, 0:rows // 2, :]) for g in range(lo, hi)], axis=1)
            sums.append(_dot(o, _bf16(wo[lo * gw // 2:hi * gw // 2, :])))

        third = (n_groups - 2) // 2
        attention(qkv, keep, pen, [lambda: None] * (n_groups - 2) + [
            lambda: groups(0, third), lambda: groups(third, 2 * third)])
        groups(2 * third, n_groups)
        return sums[0] + sums[1] + sums[2]

    def put_mem_one_layer(r, first):
        ri = jax.lax.broadcasted_iota(jnp.int32, (mt, d_model), 0)
        act = (ri < n_mem) if first else (ri >= n_mem)
        put(h_buf, 0, jnp.where(act, r, get(h_buf, 0, mt).astype(F32)))

    def project(h, g):
        return [_dot(h, _bf16(w[g])).astype(BF16) for w in w3]

    def main_step(t, use_pre, z_next=None):
        if use_pre:
            h = jnp.concatenate(
                [get(h_buf, 0, mt), get(h_buf, mt + seg, mt + 2 * seg)], axis=0)
            ps = pl.ds(pl.multiple_of((pre0 + (t - 2) * seg) // 2, 8), seg // 2)

            def qkv(g):
                return [jnp.concatenate([r[0:mt], _bf16(p[g, ps, :]), r[mt:]], axis=0)
                        for r, p in zip(project(h, g), pre)]
        else:
            qkv = functools.partial(project, get(h_buf, 0, mt + 2 * seg))
        z_old = z_buf[...]
        if not use_pre:
            put(h_buf, mt, _layernorm(x_seg(jnp.minimum(t + 1, n_seg - 1))))
        parts = []

        def finish():
            z1 = z_next
            if z1 is None:
                z = jnp.concatenate(parts, axis=1)
                z1 = z[0:seg]
                out_v[seg_rows(t - 3), :] = z[seg:2 * seg].astype(BF16)
            z_buf[...] = z1
            put(h_buf, mt + seg, _layernorm(z1))

        if z_next is None:
            attention(qkv, keep_full, pen_full, ffn_fillers(y_buf[...], parts))
            r = out_proj(mt + 2 * seg, finish)
        else:
            finish()
            r = attention_and_out_proj(qkv, keep_full, pen_full)
        put(h_buf, 0, r[0:mt])
        y_buf[0:seg, :] = x_seg(t) + r[mt:mt + seg]
        y_buf[seg:2 * seg, :] = z_old + r[mt + seg:mt + 2 * seg]
        if z_next is None:
            out_copy(t - 3, 1).start()

    x_copies[0].wait()
    mem_copy.wait()
    w3_start(1, 2 * n_groups)
    m0 = mem_v[...].astype(F32)
    m0 = jnp.concatenate([m0, m0], axis=0)
    put(h_buf, 0, m0)
    put(xpre, 0, m0)
    put(xpre, mt, _layernorm(x_seg(0)))
    put(xpre, mt + seg, _layernorm(x_seg(1))[0:half])
    for s in range(n_pre):
        put(xpre, pre0 + s * seg, _layernorm(x_seg(2 + s)))
    put(h_buf, mt, _layernorm(x_seg(2 + n_pre)))

    kq = d_model // 2
    nq = n_groups // 2

    def q_group(s, g, chunk=None):
        xs = _bf16(xpre[:, s * kq:(s + 1) * kq])
        for j in range(HG):
            cs = slice(j * dh, (j + 1) * dh)
            if chunk:
                relayout(*chunk, j, j + 1)
            r = _dot(xs, _bf16(wq[g, s * kq // 2:(s + 1) * kq // 2, cs]))
            if s == 0:
                q_acc[g, :, cs] = r
            else:
                q_pre[g, :, cs] = _pack(q_acc[g, :, cs] + r)

    def first_chunk(c):
        w3_wait(c)
        relayout(0, c)

    _loop(0, nq, first_chunk)
    _loop(0, nq, lambda g: q_group(0, g), 2)
    _loop(nq, n_groups, lambda g: q_group(0, g, (0, g)), 2, w3_wait)
    w3_start(2 * n_groups, 3 * n_groups)
    _loop(0, n_groups, lambda g: q_group(1, g, (1, g)), 2,
          lambda g: w3_wait(n_groups + g))

    def project_group(m, g, side_work=lambda j: None):
        xs = _bf16(xpre[...])
        for j in range(HG):
            cs = slice(j * dh, (j + 1) * dh)
            side_work(j)
            pre[m][g, :, cs] = _pack(_dot(xs, _bf16(w3[m][g, :, cs])))

    def precomputed(p, g, lo, hi):
        return _bf16(p[g, lo // 2:hi // 2, :])

    def k_group(g):
        project_group(1, g, lambda j: relayout(2, g, j, j + 1))

    def v_group(g):
        ps = softmaxes(precomputed(q_pre, g, 0, mt + seg), precomputed(k_pre, g, 0, mt + seg),
                       keep_one, pen_one)
        project_group(2, g)
        weigh_values(g, ps, precomputed(v_pre, g, 0, mt + seg))

    w_copies[0].start()
    w_copies[1].start()
    _loop(0, n_groups, k_group, 1, lambda g: w3_wait(2 * n_groups + g))
    w_copies[2].start()
    w_copies[3].start()
    x_copies[1].start()
    _loop(0, n_groups, v_group, 2)

    w_copies[0].wait()
    r = out_proj(mt + seg)
    put_mem_one_layer(r[0:mt], True)
    y_buf[0:seg, :] = x_seg(0) + r[mt:]

    late = _layernorm(x_seg(1))[half:].astype(BF16)
    hm = jnp.concatenate([get(h_buf, 0, mt), late], axis=0)
    r = attention_and_out_proj(
        lambda g: [jnp.concatenate(
            [a[0:mt], precomputed(p, g, mt + seg, pre0), a[mt:]], axis=0)
                   for a, p in zip(project(hm, g), pre)],
        keep_one, pen_one)
    put_mem_one_layer(r[0:mt], True)
    y_buf[seg:2 * seg, :] = x_seg(1) + r[mt:]

    w_copies[1].wait()
    w_copies[2].wait()
    w_copies[3].wait()
    y = y_buf[...]
    yn = _layernorm(y).astype(BF16)
    for c in range(n_chunks):
        ffn_up(yn, c)
    z = y + ffn_down(2 * seg, 0, d_model)
    z_buf[...] = z[0:seg]
    put(h_buf, mt + seg, _layernorm(z[0:seg]))
    main_step(2, True, z[seg:2 * seg])

    _loop(3, 2 + n_pre, lambda t: main_step(t, True))
    x_copies[1].wait()
    _loop(2 + n_pre, n_seg, lambda t: main_step(t, False))

    def second_layer_only(t):
        first = t == n_seg
        h = jnp.concatenate(
            [get(h_buf, 0, mt), get(h_buf, mt + seg, mt + 2 * seg)], axis=0)
        z_old = z_buf[...]
        parts = []

        def finish():
            z = jnp.concatenate(parts, axis=1)
            if first:
                z_buf[...] = z[0:seg]
                put(h_buf, mt + seg, _layernorm(z[0:seg]))
            out_v[(t - 3) * seg:(t - 2) * seg, :] = z[z.shape[0] - seg:].astype(BF16)

        lo = 0 if first else mt

        def qkv(g):
            return [_dot(a, _bf16(w[g])).astype(BF16) for a, w in zip((h[lo:], h, h), w3)]

        attention(qkv, keep_two, pen_two,
                  ffn_fillers(y_buf[0 if first else seg:2 * seg, :], parts))
        r = out_proj(mt + seg - lo, finish)
        if first:
            put_mem_one_layer(r[0:mt], False)
        y_buf[seg:2 * seg, :] = z_old + r[mt - lo:]
        out_copy(t - 3, 1).start()

    second_layer_only(n_seg)
    second_layer_only(n_seg + 1)
    y = y_buf[seg:2 * seg, :]
    yn = _layernorm(y).astype(BF16)
    for c in range(n_chunks):
        ffn_up(yn, c)
    z = y + ffn_down(seg, 0, d_model)
    out_v[(n_seg - 1) * seg:n_seg * seg, :] = z.astype(BF16)
    out_copy(n_seg - 1, 1).start()
    pltpu.make_async_copy(out_v, out_hbm, out_sem).wait()


@functools.partial(jax.jit, static_argnames=("A_seg_len",))
def pallas_interleave_layers__memory_aug_recurrent_mem_tr__glu_gated_geglu__prompt_kernel(
    A_x, A_mem0, A_Wq, A_Wk, A_Wv, A_Wo, A_seg_len, B_x, B_w_gate, B_w_up, B_w_down,
):
    del B_x
    _, S, Dm = A_x.shape
    _, M, _ = A_mem0.shape
    _, H, Dh = A_Wq.shape
    Df = B_w_gate.shape[1]
    seg = int(A_seg_len)
    n_seg = S // seg
    mt = 2 * M
    G = H // HG
    gw = HG * Dh
    rows = mt + 2 * seg
    pre_rows = mt + seg + seg // 2 + N_PRE * seg

    kern = functools.partial(
        _kernel, n_seg=n_seg, seg=seg, n_mem=M, n_heads=H, dh=Dh, n_pre=N_PRE)
    any_spec = pl.BlockSpec(memory_space=pl.ANY)
    out = pl.pallas_call(
        kern,
        in_specs=[any_spec] * 9,
        out_specs=any_spec,
        out_shape=jax.ShapeDtypeStruct((S, Dm), A_x.dtype),
        scratch_shapes=[
            pltpu.VMEM((S, Dm), BF16),
            pltpu.VMEM((M, Dm), BF16),
            pltpu.VMEM((3 * G, Dm // G * H, Dh), BF16),
            pltpu.VMEM((4, Dm // G * H // 8, Dh), U32),
            pltpu.VMEM((G, Dm // 2, gw), U32),
            pltpu.VMEM((G, Dm // 2, gw), U32),
            pltpu.VMEM((G, Dm // 2, gw), U32),
            pltpu.VMEM((H * Dh // 2, Dm), U32),
            pltpu.VMEM((Dm // 2, Df), U32),
            pltpu.VMEM((Dm // 2, Df), U32),
            pltpu.VMEM((Df // 2, Dm), U32),
            pltpu.VMEM((pre_rows // 2, Dm), U32),
            pltpu.VMEM((G, pre_rows, gw), F32),
            pltpu.VMEM((G, pre_rows // 2, gw), U32),
            pltpu.VMEM((G, pre_rows // 2, gw), U32),
            pltpu.VMEM((G, pre_rows // 2, gw), U32),
            pltpu.VMEM((rows // 2, Dm), U32),
            pltpu.VMEM((G, rows // 2, gw), U32),
            pltpu.VMEM((2 * seg, Dm), F32),
            pltpu.VMEM((seg, Dm), F32),
            pltpu.VMEM((seg, Df), U32),
            pltpu.VMEM((rows, rows), F32),
            pltpu.VMEM((rows, rows), F32),
            pltpu.VMEM((mt + seg, mt + seg), F32),
            pltpu.VMEM((mt + seg, mt + seg), F32),
            pltpu.VMEM((mt + seg, mt + seg), F32),
            pltpu.VMEM((mt + seg, mt + seg), F32),
            pltpu.VMEM((S, Dm), BF16),
            pltpu.SemaphoreType.DMA((3,)),
            pltpu.SemaphoreType.DMA((3 * G,)),
            pltpu.SemaphoreType.DMA((4,)),
            pltpu.SemaphoreType.DMA(()),
        ],
        compiler_params=pltpu.CompilerParams(vmem_limit_bytes=118 * 1024 * 1024),
    )(
        A_x.reshape(S, Dm), A_mem0.reshape(M, Dm),
        A_Wq.reshape(Dm * H, Dh), A_Wk.reshape(Dm * H, Dh), A_Wv.reshape(Dm * H, Dh),
        A_Wo.reshape(H * Dh, Dm), B_w_gate, B_w_up, B_w_down,
    )
    return out.reshape(1, S, Dm)
```
